```python
import jax
import jax.numpy as jnp

def _softmax(x, axis=-1):
    return jax.nn.softmax(x, axis=axis)
def _gelu(x):
    return jax.nn.gelu(x, approximate=True)
def _silu(x):
    return jax.nn.silu(x)
def _sigmoid(x):
    return jax.nn.sigmoid(x)
def _layernorm(x, axis=-1, eps=1e-5):
    m = jnp.mean(x, axis=axis, keepdims=True)
    v = jnp.var(x, axis=axis, keepdims=True)
    return (x - m) / jnp.sqrt(v + eps)
def _scatter_add(tgt, idx, src, axis=0):
    return tgt.at[idx].add(src)
def _segment_sum(src, seg, n):
    return jax.ops.segment_sum(src, seg, n)
class _Rng:
    def __init__(self, key):
        self._k = key
    def _next(self):
        self._k, sub = jax.random.split(self._k)
        return sub
    def normal(self, shape):
        return jax.random.normal(self._next(), shape, dtype=jnp.bfloat16)
    def randint(self, lo, hi, shape):
        return jax.random.randint(self._next(), shape, lo, hi, dtype=jnp.int32)
    def uniform(self, shape, lo=0.0, hi=1.0):
        return jax.random.uniform(self._next(), shape, jnp.bfloat16, lo, hi)
    def permutation(self, n):
        return jax.random.permutation(self._next(), n)


kernel_name = 'recurrent_scan__sliding_block_cached__moe_arch_mod__decode'

def setup_inputs():
    _rng = _Rng(jax.random.key(int.from_bytes(__import__("os").urandom(4), "little")))
    _w = (lambda a: (lambda t: t.astype(jnp.bfloat16) if jnp.issubdtype(t.dtype, jnp.floating) else t)(jnp.asarray(a)))
    def _A_setup():
        B, Sq, D = 1, 1, 512
        Hq, Hkv, Sk, Dh = 32, 32, 32768, 128
        assert Hq % Hkv == 0, (Hq, Hkv)
        return {
            "x": _w((lambda *s: _rng.normal(s) * 0.05)(B, Sq, D)),
            "k_cache": _w((lambda *s: _rng.normal(s) * 0.05)(B, Hkv, Sk, Dh)),
            "v_cache": _w((lambda *s: _rng.normal(s) * 0.05)(B, Hkv, Sk, Dh)),
            "wq": _w((lambda *s: _rng.normal(s) * 0.05)(D, Hq * Dh) * (D ** -0.5)),
            "wo": _w((lambda *s: _rng.normal(s) * 0.05)(Hq * Dh, D) * ((Hq * Dh) ** -0.5)),
        }
    _A_in = _A_setup()

    def _B_setup():
        B, S, D, F, C = 1, 1, 512, 1376, 1
        return {
            "x": _w((lambda *s: _rng.normal(s) * 0.05)(B, S, D)),
            "w_r": _w((lambda *s: _rng.normal(s) * 0.05)(D)),
            "w_gate": _w((lambda *s: _rng.normal(s) * 0.05)(D, F)),
            "w_up": _w((lambda *s: _rng.normal(s) * 0.05)(D, F)),
            "w_down": _w((lambda *s: _rng.normal(s) * 0.05)(F, D)),
        }
    _B_in = _B_setup()

    return {
        "A_x": _A_in["x"],
        "A_k_cache": _A_in["k_cache"],
        "A_v_cache": _A_in["v_cache"],
        "A_wq": _A_in["wq"],
        "A_wo": _A_in["wo"],
        "B_x": _B_in["x"],
        "B_w_r": _B_in["w_r"],
        "B_w_gate": _B_in["w_gate"],
        "B_w_up": _B_in["w_up"],
        "B_w_down": _B_in["w_down"],
    }

def reference(A_x, A_k_cache, A_v_cache, A_wq, A_wo, B_x, B_w_r, B_w_gate, B_w_up, B_w_down):
    def _A_ref(x, k_cache, v_cache, wq, wo):
        B, Sq, D = x.shape
        Hq, Dh = 32, 128
        Hkv, Sk = k_cache.shape[1], k_cache.shape[2]
        W = min(4096, max(256, Sk // 4))
        rep = Hq // Hkv
        q = (lambda x, *d: x.transpose(*d))((x @ wq).reshape(B, Sq, Hq, Dh), 0, 2, 1, 3)
        k = jnp.repeat(k_cache[:, :, Sk - W:, :], rep, axis=1)
        v = jnp.repeat(v_cache[:, :, Sk - W:, :], rep, axis=1)
        scores = jnp.einsum("bhqd,bhkd->bhqk", q, k) * (Dh ** -0.5)
        p = _softmax(scores, axis=-1)
        o = jnp.einsum("bhqk,bhkd->bhqd", p, v)
        return (lambda x, *d: x.transpose(*d))(o, 0, 2, 1, 3).reshape(B, Sq, Hq * Dh) @ wo

    def _B_ref(x, w_r, w_gate, w_up, w_down):
        B, S, D = x.shape
        C = 1
        r = x @ w_r
        idx = jnp.argsort(-r, axis=-1)[:, :C]
        idx_e = jnp.repeat(idx.reshape(B, C, 1), D, axis=2)
        x_sel = jnp.take_along_axis(x, idx_e, axis=1)
        g = _silu(x_sel @ w_gate)
        u = x_sel @ w_up
        y = (g * u) @ w_down
        r_sel = _sigmoid(jnp.take_along_axis(r, idx, axis=1))
        y = y * r_sel.reshape(B, C, 1)
        b_off = (jnp.arange(B) * S).reshape(B, 1)
        flat_idx = (idx + b_off).reshape(B * C)
        zero = (x * 0.0).reshape(B * S, D)
        upd = _scatter_add(zero, flat_idx, y.reshape(B * C, D), axis=0)
        return x + upd.reshape(B, S, D)

    x = A_x
    xn = _layernorm(x, axis=-1)
    s = _A_ref(xn, A_k_cache, A_v_cache, A_wq, A_wo)
    g = _silu(_B_ref(xn, B_w_r, B_w_gate, B_w_up, B_w_down))
    return x + s * g
```

```python
import jax
import jax.numpy as jnp
from jax import lax
import jax.experimental.pallas as pl
import jax.experimental.pallas.tpu as pltpu

_HQ = 32
_DH = 128
_EPS = 1e-5
_NT = (((1,), (1,)), ((), ()))
_NN = (((1,), (0,)), ((), ()))
_WO_CHUNKS = (2048, 1024, 512, 256, 128, 128)


def _sigmoid(x):
    return 1.0 / (1.0 + jnp.exp(-x))


def _make_kernel(D, F, SK, W):
    scale = _DH ** -0.5
    f32, bf16 = jnp.float32, jnp.bfloat16
    wo_off = [sum(_WO_CHUNKS[:i]) for i in range(len(_WO_CHUNKS))]
    S_WQ, S_X, S_WR, S_WG, S_WU, S_WD = range(6)
    S_KV = 6
    S_WO = S_KV + 2 * _HQ
    n_sems = S_WO + len(_WO_CHUNKS)

    def kernel(x_hbm, k_hbm, v_hbm, wq_hbm, wo_hbm, wr_hbm, wg_hbm, wu_hbm, wd_hbm,
               o_ref,
               xb, wrb, wqb, wob, wgb, wub, wdb, kb, vb, qs, os_,
               sem):
        def kcopy(h):
            return pltpu.make_async_copy(
                k_hbm.at[0, h, pl.ds(SK - W, W), :], kb.at[h], sem.at[S_KV + 2 * h])

        def vcopy(h):
            return pltpu.make_async_copy(
                v_hbm.at[0, h, pl.ds(SK - W, W), :], vb.at[h], sem.at[S_KV + 2 * h + 1])

        def wocopy(c):
            rows = pl.ds(wo_off[c], _WO_CHUNKS[c])
            return pltpu.make_async_copy(wo_hbm.at[rows, :], wob.at[rows, :], sem.at[S_WO + c])

        c_wq = pltpu.make_async_copy(wq_hbm, wqb, sem.at[S_WQ])
        c_x = pltpu.make_async_copy(x_hbm, xb, sem.at[S_X])
        c_wr = pltpu.make_async_copy(wr_hbm, wrb, sem.at[S_WR])
        c_wg = pltpu.make_async_copy(wg_hbm, wgb, sem.at[S_WG])
        c_wu = pltpu.make_async_copy(wu_hbm, wub, sem.at[S_WU])
        c_wd = pltpu.make_async_copy(wd_hbm, wdb, sem.at[S_WD])

        for c in (c_wq, c_x, c_wr, c_wg, c_wu, c_wd):
            c.start()
        for h in range(_HQ):
            kcopy(h).start()
            vcopy(h).start()
        for c in range(len(_WO_CHUNKS)):
            wocopy(c).start()

        c_x.wait()
        x = xb[0].astype(f32)
        mu = jnp.mean(x, axis=-1, keepdims=True)
        xc = x - mu
        var = jnp.mean(xc * xc, axis=-1, keepdims=True)
        xn = xc / jnp.sqrt(var + _EPS)
        xn16 = xn.astype(bf16)
        xn8 = jnp.broadcast_to(xn16, (8, D))

        c_wq.wait()
        q = lax.dot_general(xn8, wqb[...], _NN, preferred_element_type=f32)
        for h in range(_HQ):
            qs[h] = q[:, h * _DH:(h + 1) * _DH].astype(bf16)

        c_wr.wait()
        xnf = xn16.astype(f32)
        wr = wrb[...].astype(f32).reshape(1, D)
        r = jnp.sum(xnf * wr, axis=-1, keepdims=True)
        c_wg.wait()
        gpre = lax.dot_general(xn8, wgb[...], _NT, preferred_element_type=f32)
        c_wu.wait()
        u = lax.dot_general(xn8, wub[...], _NT, preferred_element_type=f32)
        hmid = (gpre * _sigmoid(gpre) * u).astype(bf16)
        c_wd.wait()
        y = lax.dot_general(hmid, wdb[...], _NN, preferred_element_type=f32)
        b_out = xnf + y[0:1, :] * _sigmoid(r)
        gate = b_out * _sigmoid(b_out)

        def head(h, carry):
            kcopy(h).wait()
            s = lax.dot_general(qs[h], kb[h], _NT, preferred_element_type=f32)
            m = jnp.max(s, axis=-1, keepdims=True)
            p = jnp.exp((s - m) * scale)
            l = jnp.sum(p, axis=-1, keepdims=True)
            vcopy(h).wait()
            o = lax.dot_general(p.astype(bf16), vb[h], _NN, preferred_element_type=f32)
            os_[h] = (o / l).astype(bf16)
            return carry

        lax.fori_loop(0, _HQ, head, 0)

        acc = jnp.zeros((8, D), f32)
        for c, n in enumerate(_WO_CHUNKS):
            h0 = wo_off[c] // _DH
            oc = jnp.concatenate([os_[h0 + i] for i in range(n // _DH)], axis=1)
            wocopy(c).wait()
            acc = acc + lax.dot_general(
                oc, wob[pl.ds(wo_off[c], n), :], _NN, preferred_element_type=f32)

        o_ref[0] = (x + acc[0:1, :] * gate).astype(o_ref.dtype)

    return kernel, n_sems


@jax.jit
def pallas_recurrent_scan__sliding_block_cached__moe_arch_mod__decode_kernel(
    A_x: jax.Array,
    A_k_cache: jax.Array,
    A_v_cache: jax.Array,
    A_wq: jax.Array,
    A_wo: jax.Array,
    B_x: jax.Array,
    B_w_r: jax.Array,
    B_w_gate: jax.Array,
    B_w_up: jax.Array,
    B_w_down: jax.Array,
):
    B, Sq, D = A_x.shape
    _, Hkv, SK, Dh = A_k_cache.shape
    F = B_w_gate.shape[1]
    assert B == 1 and Sq == 1 and Hkv == _HQ and Dh == _DH
    W = min(4096, max(256, SK // 4))
    bf16 = jnp.bfloat16
    hbm = pl.BlockSpec(memory_space=pltpu.HBM)
    kernel, n_sems = _make_kernel(D, F, SK, W)

    return pl.pallas_call(
        kernel,
        out_shape=jax.ShapeDtypeStruct((B, Sq, D), A_x.dtype),
        in_specs=[hbm] * 9,
        out_specs=pl.BlockSpec(memory_space=pltpu.VMEM),
        scratch_shapes=[
            pltpu.VMEM((1, 1, D), bf16),
            pltpu.VMEM((D,), bf16),
            pltpu.VMEM((D, _HQ * _DH), bf16),
            pltpu.VMEM((_HQ * _DH, D), bf16),
            pltpu.VMEM((F, D), bf16),
            pltpu.VMEM((F, D), bf16),
            pltpu.VMEM((F, D), bf16),
            pltpu.VMEM((_HQ, W, _DH), bf16),
            pltpu.VMEM((_HQ, W, _DH), bf16),
            pltpu.VMEM((_HQ, 8, _DH), bf16),
            pltpu.VMEM((_HQ, 8, _DH), bf16),
            pltpu.SemaphoreType.DMA((n_sems,)),
        ],
        compiler_params=pltpu.CompilerParams(
            vmem_limit_bytes=100 * 1024 * 1024,
            disable_semaphore_checks=True,
        ),
    )(A_x, A_k_cache, A_v_cache, A_wq, A_wo, B_w_r, B_w_gate.T, B_w_up.T, B_w_down)
```

```python
import functools
import jax
import jax.numpy as jnp
from jax import lax
import jax.experimental.pallas as pl
import jax.experimental.pallas.tpu as pltpu

_HQ = 32
_DH = 128
_EPS = 1e-5
_NT = (((1,), (1,)), ((), ()))
_NN = (((1,), (0,)), ((), ()))

CFG = dict(G=4, lag=2, compute=True, scopes=False, wo_tail=(1024, 512, 256, 128, 128), unroll=4)


def _sigmoid(x):
    return 1.0 / (1.0 + jnp.exp(-x))


def _make_kernel(D, F, SK, W, cfg):
    scale = _DH ** -0.5
    f32, bf16 = jnp.float32, jnp.bfloat16
    G = cfg['G']
    NG = _HQ // G
    CR = 128
    NC = W // CR
    WR = 32
    HD = _HQ * _DH
    half = HD // 2
    wo_tail = cfg['wo_tail']
    assert sum(wo_tail) == half
    do_compute = cfg['compute']

    S_X, S_WR, S_WQ, S_WG, S_WU, S_WD = range(6)
    S_K = 6
    S_V = S_K + _HQ
    S_WO = S_V + _HQ
    wo_chunks = [(0, half // 2), (half // 2, half // 2)]
    off = half
    for n in wo_tail:
        wo_chunks.append((off, n)); off += n
    n_sems = S_WO + len(wo_chunks)

    def kernel(x_hbm, k_hbm, v_hbm, wq_hbm, wo_hbm, wr_hbm, wg_hbm, wu_hbm, wd_hbm,
               o_ref,
               xb, wrb, wqb, wob, wgb, wub, wdb, kb, vb, qs, ps, ls, os_, acc_ref,
               sem):
        def whole(buf, s):
            return pltpu.make_async_copy(buf, buf, sem.at[s])

        def issue_w(i, carry):
            for u in range(3):
                j = 3 * i + u
                s4, r = j % 4, j // 4
                row = pl.multiple_of(s4 * 128 + (r // 2) * 8, 8)
                col = pl.multiple_of((r % 2) * half, half)

                @pl.when(j < 128)
                def _():
                    pltpu.make_async_copy(
                        wq_hbm.at[pl.ds(row, 8), pl.ds(col, half)],
                        wqb.at[pl.ds(row, 8), pl.ds(col, half)], sem.at[S_WQ]).start(priority=0)
                src, dst, s = ((wg_hbm, wgb, S_WG), (wu_hbm, wub, S_WU), (wd_hbm, wdb, S_WD))[u]
                rows = pl.ds(pl.multiple_of(i * WR, WR), WR)
                pltpu.make_async_copy(src.at[rows, :], dst.at[rows, :], sem.at[s]).start(priority=1)
            return carry

        def issue_kv(g, c0, n):
            def body(c, carry):
                r = pl.multiple_of(c * CR, CR)
                for j in range(G):
                    h = g * G + j
                    pltpu.make_async_copy(
                        k_hbm.at[0, h, pl.ds(SK - W + r, CR), :], kb.at[h, pl.ds(r, CR), :],
                        sem.at[S_K + h]).start(priority=0)
                    pltpu.make_async_copy(
                        v_hbm.at[0, h, pl.ds(SK - W + r, CR), :], vb.at[h, pl.ds(r, CR), :],
                        sem.at[S_V + h]).start(priority=1)
                return carry
            lax.fori_loop(c0, c0 + n, body, 0)

        def wo_sem(row):
            for ci, (o, n) in enumerate(wo_chunks):
                if o <= row < o + n:
                    return S_WO + ci

        def issue_wo(i0, n):
            for i in range(i0, i0 + n):
                for p, base in ((0, 0), (1, half)):
                    row = base + i * WR
                    rows = pl.ds(row, WR)
                    pltpu.make_async_copy(wo_hbm.at[rows, :], wob.at[rows, :],
                                          sem.at[wo_sem(row)]).start(priority=p)

        def qk(h):
            whole(kb.at[h], S_K + h).wait()
            if not do_compute:
                return
            s = lax.dot_general(qs[h], kb[h], _NT, preferred_element_type=f32)
            m = jnp.max(s, axis=-1, keepdims=True)
            p = jnp.exp((s - m) * scale)
            ls[h % G] = jnp.broadcast_to(jnp.sum(p, axis=-1, keepdims=True), (8, _DH))
            ps[h % G] = p.astype(bf16)

        def pv(h):
            whole(vb.at[h], S_V + h).wait()
            if not do_compute:
                return
            o = lax.dot_general(ps[h % G], vb[h], _NN, preferred_element_type=f32)
            os_[h] = (o / ls[h % G]).astype(bf16)

        c_x = pltpu.make_async_copy(x_hbm, xb, sem.at[S_X])
        c_wr = pltpu.make_async_copy(wr_hbm, wrb, sem.at[S_WR])
        c_x.start()
        c_wr.start()
        lax.fori_loop(0, F // WR, issue_w, 0)

        step = NC // (2 * G)
        issue_kv(0, 0, NC // 2)

        c_x.wait()
        x = xb[0].astype(f32)
        mu = jnp.mean(x, axis=-1, keepdims=True)
        xc = x - mu
        var = jnp.mean(xc * xc, axis=-1, keepdims=True)
        xn = xc / jnp.sqrt(var + _EPS)
        xn16 = xn.astype(bf16)
        xn8 = jnp.broadcast_to(xn16, (8, D))

        whole(wqb, S_WQ).wait()
        if do_compute:
            q = lax.dot_general(xn8, wqb[...], _NN, preferred_element_type=f32)
            for h in range(_HQ):
                qs[h] = q[:, h * _DH:(h + 1) * _DH].astype(bf16)
        issue_kv(0, NC // 2, NC // 4)

        c_wr.wait()
        xnf = xn16.astype(f32)
        wr = wrb[...].astype(f32).reshape(1, D)
        r = jnp.sum(xnf * wr, axis=-1, keepdims=True)
        whole(wgb, S_WG).wait()
        whole(wub, S_WU).wait()
        whole(wdb, S_WD).wait()
        if do_compute:
            gpre = lax.dot_general(xn8, wgb[...], _NT, preferred_element_type=f32)
            u = lax.dot_general(xn8, wub[...], _NT, preferred_element_type=f32)
            hmid = (gpre * _sigmoid(gpre) * u).astype(bf16)
            y = lax.dot_general(hmid, wdb[...], _NN, preferred_element_type=f32)
            b_out = xnf + y[0:1, :] * _sigmoid(r)
        else:
            b_out = xnf + r
        gate = b_out * _sigmoid(b_out)
        issue_kv(0, 3 * NC // 4, NC // 4)

        lag = cfg['lag']

        def group(g, carry):
            hp = (g - 1) * G
            issue_kv(g, 0, lag * step)

            def qk_step(j, c):
                qk(hp + j)
                issue_kv(g, (lag + j) * step, step)
                return c
            lax.fori_loop(0, G, qk_step, 0)
            rest = 2 * G - lag - G

            def pv_step(j, c):
                pv(hp + j)

                @pl.when(j < rest)
                def _():
                    issue_kv(g, (lag + G + j) * step, step)
                return c
            lax.fori_loop(0, G, pv_step, 0)
            return carry

        lax.fori_loop(1, NG, group, 0)

        nwo = half // WR
        hp = (NG - 1) * G
        issue_wo(0, nwo // 2)

        def qk_last(j, c):
            qk(hp + j)
            return c
        lax.fori_loop(0, G // 2, qk_last, 0)
        issue_wo(nwo // 2, nwo // 4)
        lax.fori_loop(G // 2, G, qk_last, 0)
        issue_wo(3 * nwo // 4, nwo // 4)

        def pv_last(j, c):
            pv(hp + j)
            return c
        lax.fori_loop(0, G, pv_last, 0)

        order = [0, 2, 1] + list(range(3, len(wo_chunks)))
        acc_ref[...] = jnp.zeros_like(acc_ref)
        for ci in order:
            o0, n = wo_chunks[ci]
            h0 = o0 // _DH
            whole(wob.at[pl.ds(o0, n), :], S_WO + ci).wait()
            if do_compute:
                oc = jnp.concatenate([os_[h0 + i] for i in range(n // _DH)], axis=1)
                acc_ref[...] += lax.dot_general(
                    oc, wob[pl.ds(o0, n), :], _NN, preferred_element_type=f32)

        o_ref[0] = (x + acc_ref[0:1, :] * gate).astype(o_ref.dtype)

    return kernel, n_sems


def build(**over):
    cfg = dict(CFG); cfg.update(over)

    @jax.jit
    def fn(A_x, A_k_cache, A_v_cache, A_wq, A_wo, B_x, B_w_r, B_w_gate, B_w_up, B_w_down):
        B, Sq, D = A_x.shape
        _, Hkv, SK, Dh = A_k_cache.shape
        F = B_w_gate.shape[1]
        W = min(4096, max(256, SK // 4))
        bf16 = jnp.bfloat16
        hbm = pl.BlockSpec(memory_space=pltpu.HBM)
        kernel, n_sems = _make_kernel(D, F, SK, W, cfg)
        G = cfg['G']
        return pl.pallas_call(
            kernel,
            out_shape=jax.ShapeDtypeStruct((B, Sq, D), A_x.dtype),
            in_specs=[hbm] * 9,
            out_specs=pl.BlockSpec(memory_space=pltpu.VMEM),
            scratch_shapes=[
                pltpu.VMEM((1, 1, D), bf16),
                pltpu.VMEM((D,), bf16),
                pltpu.VMEM((D, _HQ * _DH), bf16),
                pltpu.VMEM((_HQ * _DH, D), bf16),
                pltpu.VMEM((F, D), bf16),
                pltpu.VMEM((F, D), bf16),
                pltpu.VMEM((F, D), bf16),
                pltpu.VMEM((_HQ, W, _DH), bf16),
                pltpu.VMEM((_HQ, W, _DH), bf16),
                pltpu.VMEM((_HQ, 8, _DH), bf16),
                pltpu.VMEM((G, 8, W), bf16),
                pltpu.VMEM((G, 8, _DH), jnp.float32),
                pltpu.VMEM((_HQ, 8, _DH), bf16),
                pltpu.VMEM((8, D), jnp.float32),
                pltpu.SemaphoreType.DMA((n_sems,)),
            ],
            compiler_params=pltpu.CompilerParams(
                vmem_limit_bytes=100 * 1024 * 1024,
                disable_semaphore_checks=True,
                disable_bounds_checks=cfg.get('nobounds', False),
            ),
        )(A_x, A_k_cache, A_v_cache, A_wq, A_wo, B_w_r, B_w_gate.T, B_w_up.T, B_w_down)
    return fn

pallas_recurrent_scan__sliding_block_cached__moe_arch_mod__decode_kernel = build()
```

```python
import jax
import jax.numpy as jnp
from jax import lax
import jax.experimental.pallas as pl
import jax.experimental.pallas.tpu as pltpu

_HQ = 32
_DH = 128
_EPS = 1e-5
_NT = (((1,), (1,)), ((), ()))
_NN = (((1,), (0,)), ((), ()))

CFG = dict(lag=2, compute=True, scopes=False, warm=0, unroll=2, wo_strided=True)


def _sigmoid(x):
    return 1.0 / (1.0 + jnp.exp(-x))


def _make_kernel(D, F, SK, W, cfg):
    scale = _DH ** -0.5
    f32, bf16 = jnp.float32, jnp.bfloat16
    G = 4
    NG = _HQ // G
    CR = 32
    NC = W // CR
    WR = 32
    HD = _HQ * _DH
    half = HD // 2
    do_compute = cfg['compute']

    S_X, S_WR, S_WQ, S_WG, S_WU, S_WD = range(6)
    S_K = 6
    S_V = S_K + NG
    S_WO = S_V + NG
    S_A0, S_A1, S_B0, S_B1, S_BL = S_WO, S_WO + 1, S_WO + 2, S_WO + 3, S_WO + 4
    n_sems = S_BL + 4

    def kernel(x_hbm, k_hbm, v_hbm, wq_hbm, wo_hbm, wr_hbm, wg_hbm, wu_hbm, wd_hbm,
               o_ref,
               xb, wrb, wqb, wob, wgb, wub, wdb, kb, vb, qs, ps, ls, os_, acc_ref,
               sem):
        def whole(buf, s):
            return pltpu.make_async_copy(buf, buf, sem.at[s])

        def issue_w(i, p0):
            for u in range(3):
                j = 3 * i + u
                s4, r = j % 4, j // 4
                row = pl.multiple_of(s4 * 128 + (r // 2) * 8, 8)
                col = pl.multiple_of((r % 2) * half, half)

                @pl.when(j < 128)
                def _():
                    pltpu.make_async_copy(
                        wq_hbm.at[pl.ds(row, 8), pl.ds(col, half)],
                        wqb.at[pl.ds(row, 8), pl.ds(col, half)], sem.at[S_WQ]).start(priority=p0)
                src, dst, s = ((wg_hbm, wgb, S_WG), (wu_hbm, wub, S_WU), (wd_hbm, wdb, S_WD))[u]
                rows = pl.ds(pl.multiple_of(i * WR, WR), WR)
                pltpu.make_async_copy(src.at[rows, :], dst.at[rows, :], sem.at[s]).start(priority=1)

        def issue_kv(g, c0, n):
            heads = pl.ds(g * G, G)

            def body(c, carry):
                r = pl.multiple_of(c * CR, CR)
                pltpu.make_async_copy(
                    k_hbm.at[0, heads, pl.ds(SK - W + r, CR), :], kb.at[heads, pl.ds(r, CR), :],
                    sem.at[S_K + g]).start(priority=0)
                pltpu.make_async_copy(
                    v_hbm.at[0, heads, pl.ds(SK - W + r, CR), :], vb.at[heads, pl.ds(r, CR), :],
                    sem.at[S_V + g]).start(priority=1)
                return carry
            lax.fori_loop(0, n, lambda c, carry: body(c0 + c, carry), 0, unroll=cfg['unroll'])

        def issue_wo_round(rnd):
            sa = S_A0 if rnd < 2 else S_A1

            def body(i, carry):
                rows = pl.ds(pl.multiple_of(rnd * _DH + i * 8, 8), 8)
                pltpu.make_async_copy(wo_hbm.at[pl.ds(0, 4), rows, :], wob.at[pl.ds(0, 4), rows, :],
                                      sem.at[sa]).start(priority=0)
                if rnd < 3:
                    pltpu.make_async_copy(wo_hbm.at[pl.ds(4, 4), rows, :], wob.at[pl.ds(4, 4), rows, :],
                                          sem.at[S_B0 if rnd < 2 else S_B1]).start(priority=1)
                else:
                    s = i // 4
                    rows = pl.ds(pl.multiple_of(rnd * _DH + (i % 4) * WR, WR), WR)
                    pltpu.make_async_copy(wo_hbm.at[4 + s, rows, :], wob.at[4 + s, rows, :],
                                          sem.at[S_BL + s]).start(priority=1)
                return carry
            lax.fori_loop(0, 16, body, 0, unroll=cfg['unroll'])

        def qk(h, j):
            if not do_compute:
                return
            s = lax.dot_general(qs[h], kb[h], _NT, preferred_element_type=f32)
            m = jnp.max(s, axis=-1, keepdims=True)
            p = jnp.exp((s - m) * scale)
            ls[j] = jnp.broadcast_to(jnp.sum(p, axis=-1, keepdims=True), (8, _DH))
            ps[j] = p.astype(bf16)

        def pv(h, j):
            if not do_compute:
                return
            o = lax.dot_general(ps[j], vb[h], _NN, preferred_element_type=f32)
            os_[h] = (o / ls[j]).astype(bf16)

        def wait_k(g):
            whole(kb.at[pl.ds(g * G, G)], S_K + g).wait()

        def wait_v(g):
            whole(vb.at[pl.ds(g * G, G)], S_V + g).wait()

        c_x = pltpu.make_async_copy(x_hbm, xb, sem.at[S_X])
        c_wr = pltpu.make_async_copy(wr_hbm, wrb, sem.at[S_WR])
        warm = cfg['warm']
        if warm:
            lax.fori_loop(0, warm, lambda i, c: (issue_w(i, 1), c)[1], 0)
        c_x.start(priority=1 if warm else 0)
        c_wr.start(priority=1 if warm else 0)
        lax.fori_loop(warm, F // WR, lambda i, c: (issue_w(i, 0), c)[1], 0)

        step = NC // (2 * G)
        issue_kv(0, 0, NC // 2)

        c_x.wait()
        x = xb[0].astype(f32)
        mu = jnp.mean(x, axis=-1, keepdims=True)
        xc = x - mu
        var = jnp.mean(xc * xc, axis=-1, keepdims=True)
        xn = xc / jnp.sqrt(var + _EPS)
        xn16 = xn.astype(bf16)
        xn8 = jnp.broadcast_to(xn16, (8, D))

        whole(wqb, S_WQ).wait()
        if do_compute:
            q = lax.dot_general(xn8, wqb[...], _NN, preferred_element_type=f32)
            for h in range(_HQ):
                qs[h] = q[:, h * _DH:(h + 1) * _DH].astype(bf16)
        issue_kv(0, NC // 2, NC // 4)

        c_wr.wait()
        xnf = xn16.astype(f32)
        wr = wrb[...].astype(f32).reshape(1, D)
        r = jnp.sum(xnf * wr, axis=-1, keepdims=True)
        whole(wgb, S_WG).wait()
        whole(wub, S_WU).wait()
        whole(wdb, S_WD).wait()
        if do_compute:
            gpre = lax.dot_general(xn8, wgb[...], _NT, preferred_element_type=f32)
            u = lax.dot_general(xn8, wub[...], _NT, preferred_element_type=f32)
            hmid = (gpre * _sigmoid(gpre) * u).astype(bf16)
            y = lax.dot_general(hmid, wdb[...], _NN, preferred_element_type=f32)
            b_out = xnf + y[0:1, :] * _sigmoid(r)
        else:
            b_out = xnf + r
        gate = b_out * _sigmoid(b_out)
        issue_kv(0, 3 * NC // 4, NC // 4)

        lag = cfg['lag']

        def group(g, carry):
            hp = (g - 1) * G
            issue_kv(g, 0, lag * step)
            wait_k(g - 1)

            def qk_step(j, c):
                qk(hp + j, j)
                issue_kv(g, (lag + j) * step, step)
                return c
            lax.fori_loop(0, G, qk_step, 0)
            rest = 2 * G - lag - G
            wait_v(g - 1)

            def pv_step(j, c):
                pv(hp + j, j)

                @pl.when(j < rest)
                def _():
                    issue_kv(g, (lag + G + j) * step, step)
                return c
            lax.fori_loop(0, G, pv_step, 0)
            return carry

        lax.fori_loop(1, NG, group, 0)

        hp = (NG - 1) * G
        issue_wo_round(0)
        issue_wo_round(1)
        wait_k(NG - 1)

        def qk_last(j, c):
            qk(hp + j, j)
            return c
        lax.fori_loop(0, G // 2, qk_last, 0)
        issue_wo_round(2)
        lax.fori_loop(G // 2, G, qk_last, 0)
        issue_wo_round(3)
        wait_v(NG - 1)

        def pv_last(j, c):
            pv(hp + j, j)
            return c
        lax.fori_loop(0, G, pv_last, 0)

        acc_ref[...] = jnp.zeros_like(acc_ref)

        def wo_part(s_idx, streams, r0, nr):
            rows = pl.ds(r0 * _DH, nr * _DH)
            whole(wob.at[pl.ds(streams[0], len(streams)), rows, :], s_idx).wait()
            if do_compute:
                for s in streams:
                    oc = jnp.concatenate([os_[4 * s + r0 + i] for i in range(nr)], axis=1)
                    acc_ref[...] += lax.dot_general(oc, wob[s, rows, :], _NN, preferred_element_type=f32)

        wo_part(S_A0, (0, 1, 2, 3), 0, 2)
        wo_part(S_B0, (4, 5, 6, 7), 0, 2)
        wo_part(S_A1, (0, 1, 2, 3), 2, 2)
        wo_part(S_B1, (4, 5, 6, 7), 2, 1)
        for s in range(4):
            wo_part(S_BL + s, (4 + s,), 3, 1)

        o_ref[0] = (x + acc_ref[0:1, :] * gate).astype(o_ref.dtype)

    return kernel, n_sems


def build(**over):
    cfg = dict(CFG); cfg.update(over)

    @jax.jit
    def fn(A_x, A_k_cache, A_v_cache, A_wq, A_wo, B_x, B_w_r, B_w_gate, B_w_up, B_w_down):
        B, Sq, D = A_x.shape
        _, Hkv, SK, Dh = A_k_cache.shape
        F = B_w_gate.shape[1]
        W = min(4096, max(256, SK // 4))
        bf16 = jnp.bfloat16
        hbm = pl.BlockSpec(memory_space=pltpu.HBM)
        kernel, n_sems = _make_kernel(D, F, SK, W, cfg)
        G = 4
        return pl.pallas_call(
            kernel,
            out_shape=jax.ShapeDtypeStruct((B, Sq, D), A_x.dtype),
            in_specs=[hbm] * 9,
            out_specs=pl.BlockSpec(memory_space=pltpu.VMEM),
            scratch_shapes=[
                pltpu.VMEM((1, 1, D), bf16),
                pltpu.VMEM((D,), bf16),
                pltpu.VMEM((D, _HQ * _DH), bf16),
                pltpu.VMEM((8, _HQ * _DH // 8, D), bf16),
                pltpu.VMEM((F, D), bf16),
                pltpu.VMEM((F, D), bf16),
                pltpu.VMEM((F, D), bf16),
                pltpu.VMEM((_HQ, W, _DH), bf16),
                pltpu.VMEM((_HQ, W, _DH), bf16),
                pltpu.VMEM((_HQ, 8, _DH), bf16),
                pltpu.VMEM((G, 8, W), bf16),
                pltpu.VMEM((G, 8, _DH), jnp.float32),
                pltpu.VMEM((_HQ, 8, _DH), bf16),
                pltpu.VMEM((8, D), jnp.float32),
                pltpu.SemaphoreType.DMA((n_sems,)),
            ],
            compiler_params=pltpu.CompilerParams(
                vmem_limit_bytes=100 * 1024 * 1024,
                disable_semaphore_checks=True,
                disable_bounds_checks=cfg.get('nobounds', False),
            ),
        )(A_x, A_k_cache, A_v_cache, A_wq, A_wo.reshape(8, _HQ * _DH // 8, D), B_w_r,
          B_w_gate.T, B_w_up.T, B_w_down)
    return fn

pallas_recurrent_scan__sliding_block_cached__moe_arch_mod__decode_kernel = build()
```

```python
import jax
import jax.numpy as jnp
from jax import lax
import jax.experimental.pallas as pl
import jax.experimental.pallas.tpu as pltpu

_HQ = 32
_DH = 128
_EPS = 1e-5
_NT = (((1,), (1,)), ((), ()))
_NN = (((1,), (0,)), ((), ()))

CFG = dict(ph=16, horder=(0, 2, 1, 3), lag=2, compute=True, scopes=False, warm=0, unroll=2, wo_strided=True)


def _sigmoid(x):
    return 1.0 / (1.0 + jnp.exp(-x))


def _make_kernel(D, F, SK, W, cfg):
    scale = _DH ** -0.5
    f32, bf16 = jnp.float32, jnp.bfloat16
    G = 4
    NG = _HQ // G
    CR = 128
    PH = cfg['ph']
    NR = W // CR // 2
    NC = NR
    WR = 32
    HD = _HQ * _DH
    half = HD // 2
    do_compute = cfg['compute']

    S_X, S_WR, S_WQ, S_WG, S_WU, S_WD = range(6)
    S_K = 6
    S_V = S_K + NG
    S_WO = S_V + NG
    S_A0, S_A1, S_B0, S_B1, S_BL = S_WO, S_WO + 1, S_WO + 2, S_WO + 3, S_WO + 4
    n_sems = S_BL + 4

    def kernel(x_hbm, k_hbm, v_hbm, wq_hbm, wo_hbm, wr_hbm, wg_hbm, wu_hbm, wd_hbm,
               o_ref,
               xb, wrb, wqb, wob, wgb, wub, wdb, kb, vb, qs, ps, ls, os_, acc_ref,
               sem):
        def whole(buf, s):
            return pltpu.make_async_copy(buf, buf, sem.at[s])

        def issue_w(i, p0):
            for u in range(3):
                j = 3 * i + u
                s4, r = j % 4, j // 4
                row = pl.multiple_of(s4 * 128 + (r // 2) * 8, 8)
                col = pl.multiple_of((r % 2) * half, half)

                @pl.when(j < 128)
                def _():
                    pltpu.make_async_copy(
                        wq_hbm.at[pl.ds(row, 8), pl.ds(col, half)],
                        wqb.at[pl.ds(row, 8), pl.ds(col, half)], sem.at[S_WQ]).start(priority=p0)
                src, dst, s = ((wg_hbm, wgb, S_WG), (wu_hbm, wub, S_WU), (wd_hbm, wdb, S_WD))[u]
                rows = pl.ds(pl.multiple_of(i * WR, WR), WR)
                pltpu.make_async_copy(src.at[rows, :], dst.at[rows, :], sem.at[s]).start(priority=1)

        def kv_pair(g, h, r, n):
            pltpu.make_async_copy(
                k_hbm.at[0, h, pl.ds(SK - W + r, n), :], kb.at[h, pl.ds(r, n), :],
                sem.at[S_K + g]).start(priority=0)
            pltpu.make_async_copy(
                v_hbm.at[0, h, pl.ds(SK - W + r, n), :], vb.at[h, pl.ds(r, n), :],
                sem.at[S_V + g]).start(priority=1)

        def kv_round(g, c, first=False):
            for hi in range(2):
                for j in cfg['horder']:
                    h = g * G + j
                    if first and hi == 0:
                        kv_pair(g, h, 0, CR - PH)
                    else:
                        kv_pair(g, h, pl.multiple_of((c + hi * NR) * CR - PH, 16), CR)
            if first and PH:
                kv_pair(g, pl.ds(g * G, G), W - PH, PH)

        def issue_kv(g, c0, n):
            if isinstance(c0, int) and c0 == 0:
                kv_round(g, 0, first=True)
                c0, n = 1, n - 1
            lax.fori_loop(0, n, lambda c, carry: (kv_round(g, c0 + c), carry)[1], 0)

        def issue_wo_round(rnd):
            sa = S_A0 if rnd < 2 else S_A1

            def body(i, carry):
                rows = pl.ds(pl.multiple_of(rnd * _DH + i * 8, 8), 8)
                pltpu.make_async_copy(wo_hbm.at[pl.ds(0, 4), rows, :], wob.at[pl.ds(0, 4), rows, :],
                                      sem.at[sa]).start(priority=0)
                if rnd < 3:
                    pltpu.make_async_copy(wo_hbm.at[pl.ds(4, 4), rows, :], wob.at[pl.ds(4, 4), rows, :],
                                          sem.at[S_B0 if rnd < 2 else S_B1]).start(priority=1)
                else:
                    s = i // 4
                    rows = pl.ds(pl.multiple_of(rnd * _DH + (i % 4) * WR, WR), WR)
                    pltpu.make_async_copy(wo_hbm.at[4 + s, rows, :], wob.at[4 + s, rows, :],
                                          sem.at[S_BL + s]).start(priority=1)
                return carry
            lax.fori_loop(0, 16, body, 0, unroll=cfg['unroll'])

        def qk(h, j):
            if not do_compute:
                return
            s = lax.dot_general(qs[h], kb[h], _NT, preferred_element_type=f32)
            m = jnp.max(s, axis=-1, keepdims=True)
            p = jnp.exp((s - m) * scale)
            ls[j] = jnp.broadcast_to(jnp.sum(p, axis=-1, keepdims=True), (8, _DH))
            ps[j] = p.astype(bf16)

        def pv(h, j):
            if not do_compute:
                return
            o = lax.dot_general(ps[j], vb[h], _NN, preferred_element_type=f32)
            os_[h] = (o / ls[j]).astype(bf16)

        def wait_k(g):
            whole(kb.at[pl.ds(g * G, G)], S_K + g).wait()

        def wait_v(g):
            whole(vb.at[pl.ds(g * G, G)], S_V + g).wait()

        c_x = pltpu.make_async_copy(x_hbm, xb, sem.at[S_X])
        c_wr = pltpu.make_async_copy(wr_hbm, wrb, sem.at[S_WR])
        warm = cfg['warm']
        if warm:
            lax.fori_loop(0, warm, lambda i, c: (issue_w(i, 1), c)[1], 0)
        c_x.start(priority=1 if warm else 0)
        c_wr.start(priority=1 if warm else 0)
        lax.fori_loop(warm, F // WR, lambda i, c: (issue_w(i, 0), c)[1], 0)

        step = NC // (2 * G)
        issue_kv(0, 0, NC // 2)

        c_x.wait()
        x = xb[0].astype(f32)
        mu = jnp.mean(x, axis=-1, keepdims=True)
        xc = x - mu
        var = jnp.mean(xc * xc, axis=-1, keepdims=True)
        xn = xc / jnp.sqrt(var + _EPS)
        xn16 = xn.astype(bf16)
        xn8 = jnp.broadcast_to(xn16, (8, D))

        whole(wqb, S_WQ).wait()
        if do_compute:
            q = lax.dot_general(xn8, wqb[...], _NN, preferred_element_type=f32)
            for h in range(_HQ):
                qs[h] = q[:, h * _DH:(h + 1) * _DH].astype(bf16)
        issue_kv(0, NC // 2, NC // 4)

        c_wr.wait()
        xnf = xn16.astype(f32)
        wr = wrb[...].astype(f32).reshape(1, D)
        r = jnp.sum(xnf * wr, axis=-1, keepdims=True)
        whole(wgb, S_WG).wait()
        whole(wub, S_WU).wait()
        whole(wdb, S_WD).wait()
        if do_compute:
            gpre = lax.dot_general(xn8, wgb[...], _NT, preferred_element_type=f32)
            u = lax.dot_general(xn8, wub[...], _NT, preferred_element_type=f32)
            hmid = (gpre * _sigmoid(gpre) * u).astype(bf16)
            y = lax.dot_general(hmid, wdb[...], _NN, preferred_element_type=f32)
            b_out = xnf + y[0:1, :] * _sigmoid(r)
        else:
            b_out = xnf + r
        gate = b_out * _sigmoid(b_out)
        issue_kv(0, 3 * NC // 4, NC // 4)

        lag = cfg['lag']

        def group(g, carry):
            hp = (g - 1) * G
            issue_kv(g, 0, lag * step)
            wait_k(g - 1)

            def qk_step(j, c):
                qk(hp + j, j)
                issue_kv(g, (lag + j) * step, step)
                return c
            lax.fori_loop(0, G, qk_step, 0)
            rest = 2 * G - lag - G
            wait_v(g - 1)

            def pv_step(j, c):
                pv(hp + j, j)

                @pl.when(j < rest)
                def _():
                    issue_kv(g, (lag + G + j) * step, step)
                return c
            lax.fori_loop(0, G, pv_step, 0)
            return carry

        lax.fori_loop(1, NG, group, 0)

        hp = (NG - 1) * G
        issue_wo_round(0)
        issue_wo_round(1)
        wait_k(NG - 1)

        def qk_last(j, c):
            qk(hp + j, j)
            return c
        lax.fori_loop(0, G // 2, qk_last, 0)
        issue_wo_round(2)
        lax.fori_loop(G // 2, G, qk_last, 0)
        issue_wo_round(3)
        wait_v(NG - 1)

        def pv_last(j, c):
            pv(hp + j, j)
            return c
        lax.fori_loop(0, G, pv_last, 0)

        acc_ref[...] = jnp.zeros_like(acc_ref)

        def wo_part(s_idx, streams, r0, nr):
            rows = pl.ds(r0 * _DH, nr * _DH)
            whole(wob.at[pl.ds(streams[0], len(streams)), rows, :], s_idx).wait()
            if do_compute:
                for s in streams:
                    oc = jnp.concatenate([os_[4 * s + r0 + i] for i in range(nr)], axis=1)
                    acc_ref[...] += lax.dot_general(oc, wob[s, rows, :], _NN, preferred_element_type=f32)

        wo_part(S_A0, (0, 1, 2, 3), 0, 2)
        wo_part(S_B0, (4, 5, 6, 7), 0, 2)
        wo_part(S_A1, (0, 1, 2, 3), 2, 2)
        wo_part(S_B1, (4, 5, 6, 7), 2, 1)
        for s in range(4):
            wo_part(S_BL + s, (4 + s,), 3, 1)

        o_ref[0] = (x + acc_ref[0:1, :] * gate).astype(o_ref.dtype)

    return kernel, n_sems


def build(**over):
    cfg = dict(CFG); cfg.update(over)

    @jax.jit
    def fn(A_x, A_k_cache, A_v_cache, A_wq, A_wo, B_x, B_w_r, B_w_gate, B_w_up, B_w_down):
        B, Sq, D = A_x.shape
        _, Hkv, SK, Dh = A_k_cache.shape
        F = B_w_gate.shape[1]
        W = min(4096, max(256, SK // 4))
        bf16 = jnp.bfloat16
        hbm = pl.BlockSpec(memory_space=pltpu.HBM)
        kernel, n_sems = _make_kernel(D, F, SK, W, cfg)
        G = 4
        return pl.pallas_call(
            kernel,
            out_shape=jax.ShapeDtypeStruct((B, Sq, D), A_x.dtype),
            in_specs=[hbm] * 9,
            out_specs=pl.BlockSpec(memory_space=pltpu.VMEM),
            scratch_shapes=[
                pltpu.VMEM((1, 1, D), bf16),
                pltpu.VMEM((D,), bf16),
                pltpu.VMEM((D, _HQ * _DH), bf16),
                pltpu.VMEM((8, _HQ * _DH // 8, D), bf16),
                pltpu.VMEM((F, D), bf16),
                pltpu.VMEM((F, D), bf16),
                pltpu.VMEM((F, D), bf16),
                pltpu.VMEM((_HQ, W, _DH), bf16),
                pltpu.VMEM((_HQ, W, _DH), bf16),
                pltpu.VMEM((_HQ, 8, _DH), bf16),
                pltpu.VMEM((G, 8, W), bf16),
                pltpu.VMEM((G, 8, _DH), jnp.float32),
                pltpu.VMEM((_HQ, 8, _DH), bf16),
                pltpu.VMEM((8, D), jnp.float32),
                pltpu.SemaphoreType.DMA((n_sems,)),
            ],
            compiler_params=pltpu.CompilerParams(
                vmem_limit_bytes=100 * 1024 * 1024,
                disable_semaphore_checks=True,
                disable_bounds_checks=cfg.get('nobounds', False),
            ),
        )(A_x, A_k_cache, A_v_cache, A_wq, A_wo.reshape(8, _HQ * _DH // 8, D), B_w_r,
          B_w_gate.T, B_w_up.T, B_w_down)
    return fn

pallas_recurrent_scan__sliding_block_cached__moe_arch_mod__decode_kernel = build()
```

```python
import jax
import jax.numpy as jnp
from jax import lax
import jax.experimental.pallas as pl
import jax.experimental.pallas.tpu as pltpu

_HQ = 32
_DH = 128
_EPS = 1e-5
_NT = (((1,), (1,)), ((), ()))
_NN = (((1,), (0,)), ((), ()))

CFG = dict(vpu_tail=True, head='0011111111111111111111111111', small_at=63, SA=(0, 1, 2, 3), SB=(4, 5, 6, 7), ph=16, horder=(0, 2, 1, 3), lag=2, compute=True, scopes=False, warm=0, unroll=2, wo_strided=True)


def _sigmoid(x):
    return 1.0 / (1.0 + jnp.exp(-x))


def _make_kernel(D, F, SK, W, cfg):
    scale = _DH ** -0.5
    f32, bf16 = jnp.float32, jnp.bfloat16
    G = 4
    NG = _HQ // G
    CR = 128
    PH = cfg['ph']
    NR = W // CR // 2
    NC = NR
    WR = 32
    HD = _HQ * _DH
    half = HD // 2
    do_compute = cfg['compute']

    S_X, S_WR, S_WQ, S_WG, S_WU, S_WD = range(6)
    S_K = 6
    S_V = S_K + NG
    S_WO = S_V + NG
    S_A0, S_A1, S_B0, S_B1, S_BL = S_WO, S_WO + 1, S_WO + 2, S_WO + 3, S_WO + 4
    S_BP = S_BL + 3
    n_sems = S_BP + 4
    SA, SB = cfg['SA'], cfg['SB']

    def kernel(x_hbm, k_hbm, v_hbm, wq_hbm, wo_hbm, wr_hbm, wg_hbm, wu_hbm, wd_hbm,
               o_ref,
               xb, wrb, wqb, wob, wgb, wub, wdb, kb, vb, qs, ps, ls, os_, acc_ref, fin,
               sem):
        def whole(buf, s):
            return pltpu.make_async_copy(buf, buf, sem.at[s])

        def issue_w():
            ffn = ((wg_hbm, wgb, S_WG), (wu_hbm, wub, S_WU), (wd_hbm, wdb, S_WD))
            copies = []
            for j in range(3 * (F // WR)):
                if j < 2 * D // 8:
                    s4, r = j % 4, j // 4
                    blk = (pl.ds(s4 * (D // 4) + (r // 2) * 8, 8), pl.ds((r % 2) * half, half))
                    copies.append(pltpu.make_async_copy(wq_hbm.at[blk], wqb.at[blk], sem.at[S_WQ]))
                src, dst, s = ffn[j % 3]
                rows = pl.ds((j // 3) * WR, WR)
                copies.append(pltpu.make_async_copy(src.at[rows, :], dst.at[rows, :], sem.at[s]))
            head = cfg['head']
            for i, c in enumerate(copies):
                c.start(priority=int(head[i]) if i < len(head) else i % 2)
                if i == cfg['small_at']:
                    c_x.start()
                    c_wr.start()

        def kv_pair(g, h, r, n):
            pltpu.make_async_copy(
                k_hbm.at[0, h, pl.ds(SK - W + r, n), :], kb.at[h, pl.ds(r, n), :],
                sem.at[S_K + g]).start(priority=0)
            pltpu.make_async_copy(
                v_hbm.at[0, h, pl.ds(SK - W + r, n), :], vb.at[h, pl.ds(r, n), :],
                sem.at[S_V + g]).start(priority=1)

        def kv_round(g, c, first=False):
            for hi in range(2):
                for j in cfg['horder']:
                    h = g * G + j
                    if first and hi == 0:
                        kv_pair(g, h, 0, CR - PH)
                    else:
                        kv_pair(g, h, pl.multiple_of((c + hi * NR) * CR - PH, 16), CR)
            if first and PH:
                kv_pair(g, pl.ds(g * G, G), W - PH, PH)

        def issue_kv(g, c0, n):
            if isinstance(c0, int) and c0 == 0:
                kv_round(g, 0, first=True)
                c0, n = 1, n - 1
            lax.fori_loop(0, n, lambda c, carry: (kv_round(g, c0 + c), carry)[1], 0)

        def issue_wo_round(rnd):
            for i in range(16):
                rows = pl.ds(rnd * _DH + (i // 4) * WR, WR)
                s = SA[i % 4]
                pltpu.make_async_copy(wo_hbm.at[s, rows, :], wob.at[s, rows, :],
                                      sem.at[S_A0 if rnd < 2 else S_A1]).start(priority=0)
                if rnd < 3:
                    s, si = SB[i % 4], (S_B0 if rnd < 2 else S_B1)
                else:
                    s, si = SB[i // 4], (S_BL + i // 4 if i < 12 or not cfg['vpu_tail'] else S_BP + i % 4)
                    rows = pl.ds(rnd * _DH + (i % 4) * WR, WR)
                pltpu.make_async_copy(wo_hbm.at[s, rows, :], wob.at[s, rows, :],
                                      sem.at[si]).start(priority=1)

        def qk(h, j):
            if not do_compute:
                return
            s = lax.dot_general(qs[h], kb[h], _NT, preferred_element_type=f32)
            m = jnp.max(s, axis=-1, keepdims=True)
            p = jnp.exp((s - m) * scale)
            ls[j] = jnp.broadcast_to(jnp.sum(p, axis=-1, keepdims=True), (8, _DH))
            ps[j] = p.astype(bf16)

        def pv(h, j):
            if not do_compute:
                return
            o = lax.dot_general(ps[j], vb[h], _NN, preferred_element_type=f32)
            os_[h] = (o / ls[j]).astype(bf16)

        def wait_k(g):
            whole(kb.at[pl.ds(g * G, G)], S_K + g).wait()

        def wait_v(g):
            whole(vb.at[pl.ds(g * G, G)], S_V + g).wait()

        c_x = pltpu.make_async_copy(x_hbm, xb, sem.at[S_X])
        c_wr = pltpu.make_async_copy(wr_hbm, wrb, sem.at[S_WR])
        issue_w()

        step = NC // (2 * G)
        issue_kv(0, 0, NC // 2)

        c_x.wait()
        x = xb[0].astype(f32)
        mu = jnp.mean(x, axis=-1, keepdims=True)
        xc = x - mu
        var = jnp.mean(xc * xc, axis=-1, keepdims=True)
        xn = xc / jnp.sqrt(var + _EPS)
        xn16 = xn.astype(bf16)
        xn8 = jnp.broadcast_to(xn16, (8, D))

        whole(wqb, S_WQ).wait()
        if do_compute:
            q = lax.dot_general(xn8, wqb[...], _NN, preferred_element_type=f32)
            for h in range(_HQ):
                qs[h] = q[:, h * _DH:(h + 1) * _DH].astype(bf16)
        issue_kv(0, NC // 2, NC // 4)

        c_wr.wait()
        xnf = xn16.astype(f32)
        wr = wrb[...].astype(f32).reshape(1, D)
        r = jnp.sum(xnf * wr, axis=-1, keepdims=True)
        whole(wgb, S_WG).wait()
        whole(wub, S_WU).wait()
        whole(wdb, S_WD).wait()
        if do_compute:
            gpre = lax.dot_general(xn8, wgb[...], _NT, preferred_element_type=f32)
            u = lax.dot_general(xn8, wub[...], _NT, preferred_element_type=f32)
            hmid = (gpre * _sigmoid(gpre) * u).astype(bf16)
            y = lax.dot_general(hmid, wdb[...], _NN, preferred_element_type=f32)
            b_out = xnf + y[0:1, :] * _sigmoid(r)
        else:
            b_out = xnf + r
        gate = b_out * _sigmoid(b_out)
        issue_kv(0, 3 * NC // 4, NC // 4)

        lag = cfg['lag']

        def group(g, carry):
            hp = (g - 1) * G
            issue_kv(g, 0, lag * step)
            wait_k(g - 1)

            def qk_step(j, c):
                qk(hp + j, j)
                issue_kv(g, (lag + j) * step, step)
                return c
            lax.fori_loop(0, G, qk_step, 0)
            rest = 2 * G - lag - G
            wait_v(g - 1)

            def pv_step(j, c):
                pv(hp + j, j)

                @pl.when(j < rest)
                def _():
                    issue_kv(g, (lag + G + j) * step, step)
                return c
            lax.fori_loop(0, G, pv_step, 0)
            return carry

        lax.fori_loop(1, NG, group, 0)

        hp = (NG - 1) * G
        issue_wo_round(0)
        issue_wo_round(1)
        wait_k(NG - 1)

        def qk_last(j, c):
            qk(hp + j, j)
            return c
        lax.fori_loop(0, G // 2, qk_last, 0)
        issue_wo_round(2)
        lax.fori_loop(G // 2, G, qk_last, 0)
        issue_wo_round(3)
        wait_v(NG - 1)

        def pv_last(j, c):
            pv(hp + j, j)
            return c
        lax.fori_loop(0, G, pv_last, 0)

        acc_ref[...] = jnp.zeros_like(acc_ref)

        def wo_part(s_idx, streams, r0, nr):
            rows = pl.ds(r0 * _DH, nr * _DH)
            whole(wob.at[pl.ds(streams[0], len(streams)), rows, :], s_idx).wait()
            if do_compute:
                for s in streams:
                    oc = jnp.concatenate([os_[4 * s + r0 + i] for i in range(nr)], axis=1)
                    acc_ref[...] += lax.dot_general(oc, wob[s, rows, :], _NN, preferred_element_type=f32)

        fin[0] = jnp.broadcast_to(x, (8, D))
        fin[1] = jnp.broadcast_to(gate, (8, D))
        hl = 4 * SB[3] + 3
        if cfg['vpu_tail']:
            ocol = jnp.broadcast_to(os_[hl][0:1, :].astype(f32), (_DH, _DH)).T

        wo_part(S_A0, SA, 0, 2)
        wo_part(S_B0, SB, 0, 2)
        wo_part(S_A1, SA, 2, 2)
        wo_part(S_B1, SB, 2, 1)
        for i in range(3 if cfg['vpu_tail'] else 4):
            wo_part(S_BL + i, (SB[i],), 3, 1)

        if cfg['vpu_tail']:
            base = fin[0] + acc_ref[...] * fin[1]
            part = jnp.zeros((8, D), f32)
            for i in range(4):
                rows = pl.ds(3 * _DH + i * WR, WR)
                whole(wob.at[SB[3], rows, :], S_BP + i).wait()
                for t in range(WR // 8):
                    w = wob[SB[3], pl.ds(3 * _DH + i * WR + t * 8, 8), :].astype(f32)
                    oc = ocol[i * WR + t * 8:i * WR + t * 8 + 8, :]
                    part = part + w * jnp.concatenate([oc] * (D // _DH), axis=1)
            out = base[0:1, :] + jnp.sum(part * fin[1], axis=0, keepdims=True)
        else:
            out = (fin[0] + acc_ref[...] * fin[1])[0:1, :]
        o_ref[0] = out.astype(o_ref.dtype)

    return kernel, n_sems


def build(**over):
    cfg = dict(CFG); cfg.update(over)

    @jax.jit
    def fn(A_x, A_k_cache, A_v_cache, A_wq, A_wo, B_x, B_w_r, B_w_gate, B_w_up, B_w_down):
        B, Sq, D = A_x.shape
        _, Hkv, SK, Dh = A_k_cache.shape
        F = B_w_gate.shape[1]
        W = min(4096, max(256, SK // 4))
        bf16 = jnp.bfloat16
        hbm = pl.BlockSpec(memory_space=pltpu.HBM)
        kernel, n_sems = _make_kernel(D, F, SK, W, cfg)
        G = 4
        return pl.pallas_call(
            kernel,
            out_shape=jax.ShapeDtypeStruct((B, Sq, D), A_x.dtype),
            in_specs=[hbm] * 9,
            out_specs=pl.BlockSpec(memory_space=pltpu.VMEM),
            scratch_shapes=[
                pltpu.VMEM((1, 1, D), bf16),
                pltpu.VMEM((D,), bf16),
                pltpu.VMEM((D, _HQ * _DH), bf16),
                pltpu.VMEM((8, _HQ * _DH // 8, D), bf16),
                pltpu.VMEM((F, D), bf16),
                pltpu.VMEM((F, D), bf16),
                pltpu.VMEM((F, D), bf16),
                pltpu.VMEM((_HQ, W, _DH), bf16),
                pltpu.VMEM((_HQ, W, _DH), bf16),
                pltpu.VMEM((_HQ, 8, _DH), bf16),
                pltpu.VMEM((G, 8, W), bf16),
                pltpu.VMEM((G, 8, _DH), jnp.float32),
                pltpu.VMEM((_HQ, 8, _DH), bf16),
                pltpu.VMEM((8, D), jnp.float32),
                pltpu.VMEM((2, 8, D), jnp.float32),
                pltpu.SemaphoreType.DMA((n_sems,)),
            ],
            compiler_params=pltpu.CompilerParams(
                vmem_limit_bytes=100 * 1024 * 1024,
                disable_semaphore_checks=True,
                disable_bounds_checks=cfg.get('nobounds', False),
            ),
        )(A_x, A_k_cache, A_v_cache, A_wq, A_wo.reshape(8, _HQ * _DH // 8, D), B_w_r,
          B_w_gate.T, B_w_up.T, B_w_down)
    return fn

pallas_recurrent_scan__sliding_block_cached__moe_arch_mod__decode_kernel = build()
```

```python
import jax
import jax.numpy as jnp
from jax import lax
import jax.experimental.pallas as pl
import jax.experimental.pallas.tpu as pltpu

_HQ = 32
_DH = 128
_EPS = 1e-5
_NT = (((1,), (1,)), ((), ()))
_NN = (((1,), (0,)), ((), ()))

_G = 4
_CR = 128
_PH = 16
_WR = 32
_HEAD_ORDER = (0, 2, 1, 3)
_FIRST_PRIOS = (0, 0) + (1,) * 26
_SMALL_AT = 63
_LAG = 2
_SA, _SB = (0, 1, 4, 5), (6, 7, 2, 3)
_WO_STEPS = (12, 8, 8, 8, 8, 5, 5, 5, 5)


def _sigmoid(x):
    return 1.0 / (1.0 + jnp.exp(-x))


def _make_kernel(D, F, SK, W):
    scale = _DH ** -0.5
    f32, bf16 = jnp.float32, jnp.bfloat16
    NG = _HQ // _G
    NR = W // _CR // 2
    step = NR // (2 * _G)
    HD = _HQ * _DH
    half = HD // 2
    assert D == 512 and F % _WR == 0 and NR == 2 * _G * step

    S_X, S_WR, S_WQ, S_WG, S_WU, S_WD = range(6)
    S_K = 6
    S_V = S_K + NG
    S_WO = S_V + NG

    SR = HD // 8
    parts = [(s * SR, 2 * _DH) for s in _SA + _SB]
    parts += [(s * SR + 2 * _DH, _DH) for s in _SA + _SB]
    parts += [(s * SR + 3 * _DH, _DH) for s in _SA + _SB[:3]]
    mxu_batches = ((0, 1, 2, 3), (4, 5, 6, 7), (8, 9, 10, 11), (12, 13, 14, 15),
                   (16, 17, 18, 19, 20), (21,), (22,))
    n_mxu = len(parts)
    tail0 = _SB[3] * SR + 3 * _DH
    parts += [(tail0 + i * _WR, _WR) for i in range(_DH // _WR)]
    n_sems = S_WO + len(parts)

    def wo_sem(row):
        return S_WO + [i for i, (lo, n) in enumerate(parts) if lo <= row < lo + n][0]

    def wo_blocks(lo, hi, shifted=True):
        out = []
        for r in range(lo, hi, _WR):
            if not shifted:
                out.append([(r, _WR, 0, D)])
                continue
            blk = [(r - 8, 8, D // 2, D // 2)] if r > lo else []
            if r + _WR == hi:
                blk += [(r, _WR, 0, D)]
            else:
                blk += [(r, _WR - 8, 0, D), (r + _WR - 8, 8, 0, D // 2)]
            out.append(blk)
        return out

    sa = [wo_blocks(s * SR, (s + 1) * SR) for s in _SA]
    sb = [wo_blocks(s * SR, s * SR + 3 * _DH) + wo_blocks(s * SR + 3 * _DH, (s + 1) * SR, i < 2)
          for i, s in enumerate(_SB)]
    wo_q0 = [sa[j % 4][j // 4] for j in range(64)]
    wo_q1 = [sb[j % 4][j // 4] for j in range(48)] + [sb[j // 4][12 + j % 4] for j in range(16)]
    wo_pos = [sum(_WO_STEPS[:i]) for i in range(len(_WO_STEPS) + 1)]
    assert wo_pos[-1] == 64 and tail0 // _DH < (NG - 1) * _G

    def kernel(x_hbm, k_hbm, v_hbm, wq_hbm, wo_hbm, wr_hbm, wg_hbm, wu_hbm, wd_hbm,
               o_ref,
               xb, wrb, wqb, wob, wgb, wub, wdb, kb, vb, qs, ps, ls, os_, acc_ref, fin, ocol,
               sem):
        def wait_all(buf, s):
            pltpu.make_async_copy(buf, buf, sem.at[s]).wait()

        c_x = pltpu.make_async_copy(x_hbm, xb, sem.at[S_X])
        c_wr = pltpu.make_async_copy(wr_hbm, wrb, sem.at[S_WR])

        def issue_weights():
            ffn = ((wg_hbm, wgb, S_WG), (wu_hbm, wub, S_WU), (wd_hbm, wdb, S_WD))
            copies = []
            for j in range(max(D // 4, 3 * (F // _WR))):
                if j < D // 4:
                    ix = (pl.ds((j % 4) * (D // 4) + (j // 8) * 8, 8), pl.ds((j // 4 % 2) * half, half))
                    copies.append(pltpu.make_async_copy(wq_hbm.at[ix], wqb.at[ix], sem.at[S_WQ]))
                if j < 3 * (F // _WR):
                    src, dst, s = ffn[j % 3]
                    rows = pl.ds((j // 3) * _WR, _WR)
                    copies.append(pltpu.make_async_copy(src.at[rows, :], dst.at[rows, :], sem.at[s]))
            for i, c in enumerate(copies):
                c.start(priority=_FIRST_PRIOS[i] if i < len(_FIRST_PRIOS) else i % 2)
                if i == _SMALL_AT:
                    c_x.start()
                    c_wr.start()

        def kv_pair(g, h, r, n):
            pltpu.make_async_copy(
                k_hbm.at[0, h, pl.ds(SK - W + r, n), :], kb.at[h, pl.ds(r, n), :],
                sem.at[S_K + g]).start(priority=0)
            pltpu.make_async_copy(
                v_hbm.at[0, h, pl.ds(SK - W + r, n), :], vb.at[h, pl.ds(r, n), :],
                sem.at[S_V + g]).start(priority=1)

        def kv_round(g, c, first=False):
            for hi in range(2):
                for j in _HEAD_ORDER:
                    if first and hi == 0:
                        kv_pair(g, g * _G + j, 0, _CR - _PH)
                    else:
                        kv_pair(g, g * _G + j, pl.multiple_of((c + hi * NR) * _CR - _PH, 16), _CR)
            if first:
                kv_pair(g, pl.ds(g * _G, _G), W - _PH, _PH)

        def issue_kv(g, c0, n):
            if isinstance(c0, int) and c0 == 0:
                kv_round(g, 0, first=True)
                c0, n = 1, n - 1

            def body(c, carry):
                kv_round(g, c0 + c)
                return carry
            lax.fori_loop(0, n, body, 0)

        def issue_wo(t):
            for i in range(wo_pos[t], wo_pos[t + 1]):
                for p, blk in enumerate((wo_q0[i], wo_q1[i])):
                    for r, nr, c, nc in blk:
                        ix = (pl.ds(r, nr), pl.ds(c, nc))
                        pltpu.make_async_copy(
                            wo_hbm.at[ix], wob.at[ix], sem.at[wo_sem(r)]).start(priority=p)

        def qk(h, j):
            s = lax.dot_general(qs[h], kb[h], _NT, preferred_element_type=f32)
            m = jnp.max(s, axis=-1, keepdims=True)
            p = jnp.exp((s - m) * scale)
            ls[j] = jnp.broadcast_to(jnp.sum(p, axis=-1, keepdims=True), (8, _DH))
            ps[j] = p.astype(bf16)

        def pv(h, j):
            o = lax.dot_general(ps[j], vb[h], _NN, preferred_element_type=f32)
            os_[h] = (o / ls[j]).astype(bf16)

        def wait_k(g):
            wait_all(kb.at[pl.ds(g * _G, _G)], S_K + g)

        def wait_v(g):
            wait_all(vb.at[pl.ds(g * _G, _G)], S_V + g)

        issue_weights()
        issue_kv(0, 0, NR // 2)

        c_x.wait()
        x = xb[0].astype(f32)
        mu = jnp.mean(x, axis=-1, keepdims=True)
        xc = x - mu
        var = jnp.mean(xc * xc, axis=-1, keepdims=True)
        xn16 = (xc / jnp.sqrt(var + _EPS)).astype(bf16)
        xn8 = jnp.broadcast_to(xn16, (8, D))

        wait_all(wqb, S_WQ)
        q = lax.dot_general(xn8, wqb[...], _NN, preferred_element_type=f32)
        for h in range(_HQ):
            qs[h] = q[:, h * _DH:(h + 1) * _DH].astype(bf16)
        issue_kv(0, NR // 2, NR // 4)

        c_wr.wait()
        xn = xn16.astype(f32)
        r = jnp.sum(xn * wrb[...].astype(f32).reshape(1, D), axis=-1, keepdims=True)
        wait_all(wgb, S_WG)
        wait_all(wub, S_WU)
        wait_all(wdb, S_WD)
        gpre = lax.dot_general(xn8, wgb[...], _NT, preferred_element_type=f32)
        u = lax.dot_general(xn8, wub[...], _NT, preferred_element_type=f32)
        hmid = (gpre * _sigmoid(gpre) * u).astype(bf16)
        y = lax.dot_general(hmid, wdb[...], _NN, preferred_element_type=f32)
        b_out = xn + y[0:1, :] * _sigmoid(r)
        fin[0] = jnp.broadcast_to(x, (8, D))
        fin[1] = jnp.broadcast_to(b_out * _sigmoid(b_out), (8, D))
        issue_kv(0, 3 * NR // 4, NR // 4)

        def group(g, carry):
            hp = (g - 1) * _G
            issue_kv(g, 0, _LAG * step)
            wait_k(g - 1)

            def qk_step(j, c):
                qk(hp + j, j)
                issue_kv(g, (_LAG + j) * step, step)
                return c
            lax.fori_loop(0, _G, qk_step, 0)
            wait_v(g - 1)

            def pv_step(j, c):
                pv(hp + j, j)

                @pl.when(j < _G - _LAG)
                def _():
                    issue_kv(g, (_LAG + _G + j) * step, step)
                return c
            lax.fori_loop(0, _G, pv_step, 0)
            return carry

        lax.fori_loop(1, NG, group, 0)

        hp = (NG - 1) * _G
        ocol[...] = jnp.broadcast_to(os_[tail0 // _DH][0:1, :].astype(f32), (_DH, _DH)).T

        def last(fn, t0):
            def body(j, c):
                fn(hp + j, j)
                for t in range(_G):
                    pl.when(j == t)(lambda t=t: issue_wo(t0 + t))
                return c
            lax.fori_loop(0, _G, body, 0)

        issue_wo(0)
        wait_k(NG - 1)
        last(qk, 1)
        wait_v(NG - 1)
        last(pv, 1 + _G)

        acc_ref[...] = jnp.zeros_like(acc_ref)
        for batch in mxu_batches:
            for i in batch:
                lo, n = parts[i]
                wait_all(wob.at[pl.ds(lo, n), :], S_WO + i)
            for i in batch:
                lo, n = parts[i]
                oc = jnp.concatenate([os_[lo // _DH + t] for t in range(n // _DH)], axis=1)
                acc_ref[...] += lax.dot_general(
                    oc, wob[pl.ds(lo, n), :], _NN, preferred_element_type=f32)

        base = fin[0] + acc_ref[...] * fin[1]
        part = jnp.zeros((8, D), f32)
        for i in range(n_mxu, len(parts)):
            lo, n = parts[i]
            wait_all(wob.at[pl.ds(lo, n), :], S_WO + i)
            for r0 in range(lo, lo + n, 8):
                w = wob[pl.ds(r0, 8), :].astype(f32)
                oc = ocol[pl.ds(r0 - tail0, 8), :]
                part = part + w * jnp.concatenate([oc] * (D // _DH), axis=1)
        out = base[0:1, :] + jnp.sum(part * fin[1], axis=0, keepdims=True)
        o_ref[0] = out.astype(o_ref.dtype)

    return kernel, n_sems


@jax.jit
def pallas_recurrent_scan__sliding_block_cached__moe_arch_mod__decode_kernel(
    A_x: jax.Array,
    A_k_cache: jax.Array,
    A_v_cache: jax.Array,
    A_wq: jax.Array,
    A_wo: jax.Array,
    B_x: jax.Array,
    B_w_r: jax.Array,
    B_w_gate: jax.Array,
    B_w_up: jax.Array,
    B_w_down: jax.Array,
):
    del B_x
    B, Sq, D = A_x.shape
    _, Hkv, SK, Dh = A_k_cache.shape
    F = B_w_gate.shape[1]
    assert B == 1 and Sq == 1 and Hkv == _HQ and Dh == _DH
    W = min(4096, max(256, SK // 4))
    f32, bf16 = jnp.float32, jnp.bfloat16
    kernel, n_sems = _make_kernel(D, F, SK, W)

    return pl.pallas_call(
        kernel,
        out_shape=jax.ShapeDtypeStruct((B, Sq, D), A_x.dtype),
        in_specs=[pl.BlockSpec(memory_space=pltpu.HBM)] * 9,
        out_specs=pl.BlockSpec(memory_space=pltpu.VMEM),
        scratch_shapes=[
            pltpu.VMEM((1, 1, D), bf16),
            pltpu.VMEM((D,), bf16),
            pltpu.VMEM((D, _HQ * _DH), bf16),
            pltpu.VMEM((_HQ * _DH, D), bf16),
            pltpu.VMEM((F, D), bf16),
            pltpu.VMEM((F, D), bf16),
            pltpu.VMEM((F, D), bf16),
            pltpu.VMEM((_HQ, W, _DH), bf16),
            pltpu.VMEM((_HQ, W, _DH), bf16),
            pltpu.VMEM((_HQ, 8, _DH), bf16),
            pltpu.VMEM((_G, 8, W), bf16),
            pltpu.VMEM((_G, 8, _DH), f32),
            pltpu.VMEM((_HQ, 8, _DH), bf16),
            pltpu.VMEM((8, D), f32),
            pltpu.VMEM((2, 8, D), f32),
            pltpu.VMEM((_DH, _DH), f32),
            pltpu.SemaphoreType.DMA((n_sems,)),
        ],
        compiler_params=pltpu.CompilerParams(
            vmem_limit_bytes=100 * 1024 * 1024,
            disable_semaphore_checks=True,
        ),
    )(A_x, A_k_cache, A_v_cache, A_wq, A_wo, B_w_r, B_w_gate.T, B_w_up.T, B_w_down)
```

```python
import jax
import jax.numpy as jnp
from jax import lax
import jax.experimental.pallas as pl
import jax.experimental.pallas.tpu as pltpu

_HQ = 32
_DH = 128
_EPS = 1e-5
_NT = (((1,), (1,)), ((), ()))
_NN = (((1,), (0,)), ((), ()))

_G = 4
_CR = 128
_PH = 16
_WR = 32
_HEAD_ORDER = (0, 2, 1, 3)
_FIRST_PRIOS = (0, 0) + (1,) * 20
_SMALL_AT = 63
_LAG = 2
_SA, _SB = (0, 1, 4, 5), (6, 7, 2, 3)
_WO_STEPS = (12, 8, 8, 8, 8, 5, 5, 5, 5)


def _sigmoid(x):
    return 1.0 / (1.0 + jnp.exp(-x))


def _make_kernel(D, F, SK, W):
    scale = _DH ** -0.5
    f32, bf16 = jnp.float32, jnp.bfloat16
    NG = _HQ // _G
    NR = W // _CR // 2
    step = NR // (2 * _G)
    HD = _HQ * _DH
    half = HD // 2
    assert D == 512 and F % _WR == 0 and NR == 2 * _G * step

    S_X, S_WR, S_WQ, S_WG, S_WU, S_WD = range(6)
    S_K = 6
    S_V = S_K + NG
    S_WO = S_V + NG

    SR = HD // 8
    parts = [(s * SR, 2 * _DH) for s in _SA + _SB]
    parts += [(s * SR + 2 * _DH, _DH) for s in _SA + _SB]
    parts += [(s * SR + 3 * _DH, _DH) for s in _SA + _SB[:2]]
    mxu_batches = ((0, 1, 2, 3), (4, 5, 6, 7), (8, 9, 10, 11), (12, 13, 14, 15),
                   (16, 17, 18, 19, 20), (21,))
    n_mxu = len(parts)
    tails = [s * SR + 3 * _DH for s in _SB[2:]]
    parts += [(tails[0], _DH)] + [(tails[1] + i * _WR, _WR) for i in range(_DH // _WR)]
    n_sems = S_WO + len(parts)

    def wo_sem(row):
        return S_WO + [i for i, (lo, n) in enumerate(parts) if lo <= row < lo + n][0]

    def wo_blocks(lo, hi, shifted=True):
        out = []
        for r in range(lo, hi, _WR):
            if not shifted:
                out.append([(r, _WR, 0, D)])
                continue
            blk = [(r - 8, 8, D // 2, D // 2)] if r > lo else []
            if r + _WR == hi:
                blk += [(r, _WR, 0, D)]
            else:
                blk += [(r, _WR - 8, 0, D), (r + _WR - 8, 8, 0, D // 2)]
            out.append(blk)
        return out

    sa = [wo_blocks(s * SR, (s + 1) * SR) for s in _SA]
    sb = [wo_blocks(s * SR, s * SR + 3 * _DH) + wo_blocks(s * SR + 3 * _DH, (s + 1) * SR, i < 2)
          for i, s in enumerate(_SB)]
    wo_q0 = [sa[j % 4][j // 4] for j in range(64)]
    wo_q1 = [sb[j % 4][j // 4] for j in range(48)] + [sb[j // 4][12 + j % 4] for j in range(16)]
    wo_pos = [sum(_WO_STEPS[:i]) for i in range(len(_WO_STEPS) + 1)]
    assert wo_pos[-1] == 64 and max(tails) // _DH < (NG - 1) * _G

    def kernel(x_hbm, k_hbm, v_hbm, wq_hbm, wo_hbm, wr_hbm, wg_hbm, wu_hbm, wd_hbm,
               o_ref,
               xb, wrb, wqb, wob, wgb, wub, wdb, kb, vb, qs, ps, ls, os_, acc_ref, fin, ocol,
               sem):
        def wait_all(buf, s):
            pltpu.make_async_copy(buf, buf, sem.at[s]).wait()

        c_x = pltpu.make_async_copy(x_hbm, xb, sem.at[S_X])
        c_wr = pltpu.make_async_copy(wr_hbm, wrb, sem.at[S_WR])

        def issue_weights():
            ffn = ((wg_hbm, wgb, S_WG), (wu_hbm, wub, S_WU), (wd_hbm, wdb, S_WD))
            sh = 2 * _DH
            blocks = []
            for j in range(max(D // 4, 3 * (F // _WR))):
                if j < D // 4:
                    b = (j % 8) * (D // 32) + j // 8
                    r = b // 2 * 8
                    if b % 2:
                        rects = [(r, half - sh, half)]
                    else:
                        rects = [((r - 8) % D, HD - sh, sh), (r, 0, half - sh)]
                    ixs = [(pl.ds(r0, 8), pl.ds(c0, nc)) for r0, c0, nc in rects]
                    blocks.append([pltpu.make_async_copy(wq_hbm.at[ix], wqb.at[ix], sem.at[S_WQ])
                                   for ix in ixs])
                if j < 3 * (F // _WR):
                    src, dst, s = ffn[j % 3]
                    rows = pl.ds((j // 3) * _WR, _WR)
                    blocks.append([pltpu.make_async_copy(src.at[rows, :], dst.at[rows, :], sem.at[s])])
            for i, blk in enumerate(blocks):
                for c in blk:
                    c.start(priority=_FIRST_PRIOS[i] if i < len(_FIRST_PRIOS) else i % 2)
                if i == _SMALL_AT:
                    c_x.start()
                    c_wr.start()

        def kv_pair(g, h, r, n):
            pltpu.make_async_copy(
                k_hbm.at[0, h, pl.ds(SK - W + r, n), :], kb.at[h, pl.ds(r, n), :],
                sem.at[S_K + g]).start(priority=0)
            pltpu.make_async_copy(
                v_hbm.at[0, h, pl.ds(SK - W + r, n), :], vb.at[h, pl.ds(r, n), :],
                sem.at[S_V + g]).start(priority=1)

        def kv_round(g, c, first=False):
            for hi in range(2):
                for j in _HEAD_ORDER:
                    if first and hi == 0:
                        kv_pair(g, g * _G + j, 0, _CR - _PH)
                    else:
                        kv_pair(g, g * _G + j, pl.multiple_of((c + hi * NR) * _CR - _PH, 16), _CR)
            if first:
                kv_pair(g, pl.ds(g * _G, _G), W - _PH, _PH)

        def issue_kv(g, c0, n):
            if isinstance(c0, int) and c0 == 0:
                kv_round(g, 0, first=True)
                c0, n = 1, n - 1

            def body(c, carry):
                kv_round(g, c0 + c)
                return carry
            lax.fori_loop(0, n, body, 0)

        def issue_wo(t):
            for i in range(wo_pos[t], wo_pos[t + 1]):
                for p, blk in enumerate((wo_q0[i], wo_q1[i])):
                    for r, nr, c, nc in blk:
                        ix = (pl.ds(r, nr), pl.ds(c, nc))
                        pltpu.make_async_copy(
                            wo_hbm.at[ix], wob.at[ix], sem.at[wo_sem(r)]).start(priority=p)

        def qk(h, j):
            s = lax.dot_general(qs[h], kb[h], _NT, preferred_element_type=f32)
            m = jnp.max(s, axis=-1, keepdims=True)
            p = jnp.exp((s - m) * scale)
            ls[j] = jnp.broadcast_to(jnp.sum(p, axis=-1, keepdims=True), (8, _DH))
            ps[j] = p.astype(bf16)

        def pv(h, j):
            o = lax.dot_general(ps[j], vb[h], _NN, preferred_element_type=f32)
            os_[h] = (o / ls[j]).astype(bf16)

        def wait_k(g):
            wait_all(kb.at[pl.ds(g * _G, _G)], S_K + g)

        def wait_v(g):
            wait_all(vb.at[pl.ds(g * _G, _G)], S_V + g)

        issue_weights()
        issue_kv(0, 0, NR // 2)

        c_x.wait()
        x = xb[0].astype(f32)
        mu = jnp.mean(x, axis=-1, keepdims=True)
        xc = x - mu
        var = jnp.mean(xc * xc, axis=-1, keepdims=True)
        xn16 = (xc / jnp.sqrt(var + _EPS)).astype(bf16)
        xn8 = jnp.broadcast_to(xn16, (8, D))

        wait_all(wqb, S_WQ)
        q = lax.dot_general(xn8, wqb[...], _NN, preferred_element_type=f32)
        for h in range(_HQ):
            qs[h] = q[:, h * _DH:(h + 1) * _DH].astype(bf16)
        issue_kv(0, NR // 2, NR // 4)

        c_wr.wait()
        xn = xn16.astype(f32)
        r = jnp.sum(xn * wrb[...].astype(f32).reshape(1, D), axis=-1, keepdims=True)
        wait_all(wgb, S_WG)
        wait_all(wub, S_WU)
        wait_all(wdb, S_WD)
        gpre = lax.dot_general(xn8, wgb[...], _NT, preferred_element_type=f32)
        u = lax.dot_general(xn8, wub[...], _NT, preferred_element_type=f32)
        hmid = (gpre * _sigmoid(gpre) * u).astype(bf16)
        y = lax.dot_general(hmid, wdb[...], _NN, preferred_element_type=f32)
        b_out = xn + y[0:1, :] * _sigmoid(r)
        fin[0] = jnp.broadcast_to(x, (8, D))
        fin[1] = jnp.broadcast_to(b_out * _sigmoid(b_out), (8, D))
        issue_kv(0, 3 * NR // 4, NR // 4)

        def group(g, carry):
            hp = (g - 1) * _G
            issue_kv(g, 0, _LAG * step)
            wait_k(g - 1)

            def qk_step(j, c):
                qk(hp + j, j)
                issue_kv(g, (_LAG + j) * step, step)
                return c
            lax.fori_loop(0, _G, qk_step, 0)
            wait_v(g - 1)

            def pv_step(j, c):
                pv(hp + j, j)

                @pl.when(j < _G - _LAG)
                def _():
                    issue_kv(g, (_LAG + _G + j) * step, step)
                return c
            lax.fori_loop(0, _G, pv_step, 0)
            return carry

        lax.fori_loop(1, NG, group, 0)

        hp = (NG - 1) * _G
        for i, t0 in enumerate(tails):
            ocol[i] = jnp.broadcast_to(os_[t0 // _DH][0:1, :].astype(f32), (_DH, _DH)).T

        def last(fn, t0):
            def body(j, c):
                fn(hp + j, j)
                for t in range(_G):
                    pl.when(j == t)(lambda t=t: issue_wo(t0 + t))
                return c
            lax.fori_loop(0, _G, body, 0)

        issue_wo(0)
        wait_k(NG - 1)
        last(qk, 1)
        wait_v(NG - 1)
        last(pv, 1 + _G)

        acc_ref[...] = jnp.zeros_like(acc_ref)
        for batch in mxu_batches:
            for i in batch:
                lo, n = parts[i]
                wait_all(wob.at[pl.ds(lo, n), :], S_WO + i)
            for i in batch:
                lo, n = parts[i]
                oc = jnp.concatenate([os_[lo // _DH + t] for t in range(n // _DH)], axis=1)
                acc_ref[...] += lax.dot_general(
                    oc, wob[pl.ds(lo, n), :], _NN, preferred_element_type=f32)

        base = fin[0] + acc_ref[...] * fin[1]
        part = jnp.zeros((8, D), f32)
        for i in range(n_mxu, len(parts)):
            lo, n = parts[i]
            wait_all(wob.at[pl.ds(lo, n), :], S_WO + i)
            for r0 in range(lo, lo + n, 8):
                w = wob[pl.ds(r0, 8), :].astype(f32)
                oc = ocol[min(i - n_mxu, 1), pl.ds(r0 % _DH, 8), :]
                part = part + w * jnp.concatenate([oc] * (D // _DH), axis=1)
        out = base[0:1, :] + jnp.sum(part * fin[1], axis=0, keepdims=True)
        o_ref[0] = out.astype(o_ref.dtype)

    return kernel, n_sems


@jax.jit
def pallas_recurrent_scan__sliding_block_cached__moe_arch_mod__decode_kernel(
    A_x: jax.Array,
    A_k_cache: jax.Array,
    A_v_cache: jax.Array,
    A_wq: jax.Array,
    A_wo: jax.Array,
    B_x: jax.Array,
    B_w_r: jax.Array,
    B_w_gate: jax.Array,
    B_w_up: jax.Array,
    B_w_down: jax.Array,
):
    del B_x
    B, Sq, D = A_x.shape
    _, Hkv, SK, Dh = A_k_cache.shape
    F = B_w_gate.shape[1]
    assert B == 1 and Sq == 1 and Hkv == _HQ and Dh == _DH
    W = min(4096, max(256, SK // 4))
    f32, bf16 = jnp.float32, jnp.bfloat16
    kernel, n_sems = _make_kernel(D, F, SK, W)

    return pl.pallas_call(
        kernel,
        out_shape=jax.ShapeDtypeStruct((B, Sq, D), A_x.dtype),
        in_specs=[pl.BlockSpec(memory_space=pltpu.HBM)] * 9,
        out_specs=pl.BlockSpec(memory_space=pltpu.VMEM),
        scratch_shapes=[
            pltpu.VMEM((1, 1, D), bf16),
            pltpu.VMEM((D,), bf16),
            pltpu.VMEM((D, _HQ * _DH), bf16),
            pltpu.VMEM((_HQ * _DH, D), bf16),
            pltpu.VMEM((F, D), bf16),
            pltpu.VMEM((F, D), bf16),
            pltpu.VMEM((F, D), bf16),
            pltpu.VMEM((_HQ, W, _DH), bf16),
            pltpu.VMEM((_HQ, W, _DH), bf16),
            pltpu.VMEM((_HQ, 8, _DH), bf16),
            pltpu.VMEM((_G, 8, W), bf16),
            pltpu.VMEM((_G, 8, _DH), f32),
            pltpu.VMEM((_HQ, 8, _DH), bf16),
            pltpu.VMEM((8, D), f32),
            pltpu.VMEM((2, 8, D), f32),
            pltpu.VMEM((2, _DH, _DH), f32),
            pltpu.SemaphoreType.DMA((n_sems,)),
        ],
        compiler_params=pltpu.CompilerParams(
            vmem_limit_bytes=100 * 1024 * 1024,
            disable_semaphore_checks=True,
        ),
    )(A_x, A_k_cache, A_v_cache, A_wq, A_wo, B_w_r, B_w_gate.T, B_w_up.T, B_w_down)
```

```python
import jax
import jax.numpy as jnp
from jax import lax
import jax.experimental.pallas as pl
import jax.experimental.pallas.tpu as pltpu

_HQ = 32
_DH = 128
_EPS = 1e-5
_NT = (((1,), (1,)), ((), ()))
_NN = (((1,), (0,)), ((), ()))

_G = 4
_CR = 128
_PH = 16
_WR = 32
_FIRST_PRIOS = ((0,) + (1,) * 11) * 2
_SMALL_AT = 63
_LAG = 2
_SA, _SB = (0, 1, 6, 7), (5, 4, 2, 3)
_WO_STEPS = (12, 8, 8, 8, 8, 5, 5, 5, 5)


def _sigmoid(x):
    return 1.0 / (1.0 + jnp.exp(-x))


def _make_kernel(D, F, SK, W):
    scale = _DH ** -0.5
    f32, bf16 = jnp.float32, jnp.bfloat16
    NG = _HQ // _G
    NR = W // _CR // 2
    step = NR // (2 * _G)
    HD = _HQ * _DH
    half = HD // 2
    assert D == 512 and F % _WR == 0 and 3 * (F // _WR) >= D // 4 and NR == 2 * _G * step

    S_X, S_WR, S_WQ, S_WG, S_WU, S_WD = range(6)
    S_K = 6
    S_V = S_K + NG
    S_WO = S_V + NG

    SR = HD // 8
    parts = [(s * SR, 2 * _DH) for s in _SA + _SB]
    parts += [(s * SR + 2 * _DH, _DH) for s in _SA + _SB]
    parts += [(s * SR + 3 * _DH, _DH) for s in _SA + _SB[:2]]
    mxu_batches = ((0, 1, 2, 3), (4, 5, 6, 7), (8, 9, 10, 11), (12, 13, 14, 15),
                   (16, 17, 18, 19), (20, 21))
    n_mxu = len(parts)
    tails = [s * SR + 3 * _DH for s in _SB[2:]]
    parts += [(tails[0], _DH)] + [(tails[1] + i * _WR, _WR) for i in range(_DH // _WR)]
    n_sems = S_WO + len(parts)

    def wo_sem(row):
        return S_WO + [i for i, (lo, n) in enumerate(parts) if lo <= row < lo + n][0]

    def wo_blocks(lo, hi, shifted=True):
        out = []
        for r in range(lo, hi, _WR):
            if not shifted:
                out.append([(r, _WR, 0, D)])
                continue
            blk = [(r - 8, 8, D // 2, D // 2)] if r > lo else []
            if r + _WR == hi:
                blk += [(r, _WR, 0, D)]
            else:
                blk += [(r, _WR - 8, 0, D), (r + _WR - 8, 8, 0, D // 2)]
            out.append(blk)
        return out

    sa = [wo_blocks(s * SR, (s + 1) * SR) for s in _SA]
    sb = [wo_blocks(s * SR, s * SR + 3 * _DH) + wo_blocks(s * SR + 3 * _DH, (s + 1) * SR, i < 2)
          for i, s in enumerate(_SB)]

    def round_robin(streams, lo, hi):
        turns = [[lo]] + [[b, b + 1] for b in range(lo + 1, hi - 1, 2)] + [[hi - 1]]
        return [st[b] for turn in turns for st in streams for b in turn]

    wo_q0 = round_robin(sa, 0, 16)
    wo_q1 = round_robin(sb, 0, 12) + round_robin(sb[:2], 12, 16) + sb[2][12:] + sb[3][12:]
    wo_pos = [sum(_WO_STEPS[:i]) for i in range(len(_WO_STEPS) + 1)]
    assert wo_pos[-1] == 64 and max(tails) // _DH < (NG - 1) * _G

    def kernel(x_hbm, k_hbm, v_hbm, wq_hbm, wo_hbm, wr_hbm, wg_hbm, wu_hbm, wd_hbm,
               o_ref,
               xb, wrb, wqb, wob, wgb, wub, wdb, kb, vb, qs, ps, ls, os_, acc_ref, fin, ocol,
               sem):
        def wait_all(buf, s):
            pltpu.make_async_copy(buf, buf, sem.at[s]).wait()

        c_x = pltpu.make_async_copy(x_hbm, xb, sem.at[S_X])
        c_wr = pltpu.make_async_copy(wr_hbm, wrb, sem.at[S_WR])

        def issue_weights():
            ffn = ((wd_hbm, wdb, S_WD), (wu_hbm, wub, S_WU), (wg_hbm, wgb, S_WG))
            sh, nq, nf = 2 * _DH, D // 4, F // _WR
            blocks = []
            for j in range(max(nq, 3 * nf)):
                pos = (j // 2 % 8) * (nq // 8) + j // 16 * 2 + j % 2
                if j < nq:
                    b = (pos + 1) % nq
                    r = b // 2 * 8
                    if b % 2:
                        rects = [(r, half - sh, half)]
                    else:
                        rects = [((r - 8) % D, HD - sh, sh), (r, 0, half - sh)]
                    ixs = [(pl.ds(r0, 8), pl.ds(c0, nc)) for r0, c0, nc in rects]
                    blocks.append([pltpu.make_async_copy(wq_hbm.at[ix], wqb.at[ix], sem.at[S_WQ])
                                   for ix in ixs])
                b = (pos + 2) % nq if j < nq else j
                src, dst, s = ffn[b // nf]
                rows = pl.ds(b % nf * _WR, _WR)
                blocks.append([pltpu.make_async_copy(src.at[rows, :], dst.at[rows, :], sem.at[s])])
            for i, blk in enumerate(blocks):
                for c in blk:
                    c.start(priority=_FIRST_PRIOS[i] if i < len(_FIRST_PRIOS) else i % 2)
                if i == _SMALL_AT:
                    c_x.start()
                    c_wr.start()

        def kv_pair(g, h, r, n):
            pltpu.make_async_copy(
                k_hbm.at[0, h, pl.ds(SK - W + r, n), :], kb.at[h, pl.ds(r, n), :],
                sem.at[S_K + g]).start(priority=0)
            pltpu.make_async_copy(
                v_hbm.at[0, h, pl.ds(SK - W + r, n), :], vb.at[h, pl.ds(r, n), :],
                sem.at[S_V + g]).start(priority=1)

        def kv_round(g, c, first=False):
            m = NR - 1 - (c % 2 * (NR // 2) + c // 2)
            for j in range(_G):
                if first:
                    kv_pair(g, g * _G + j, W - _CR - _PH, _CR + _PH)
                    kv_pair(g, g * _G + j, 0, _CR - _PH)
                else:
                    for e in (1, 2):
                        kv_pair(g, g * _G + j, pl.multiple_of((2 * m + e) * _CR - _PH, 16), _CR)

        def issue_kv(g, c0, n):
            if isinstance(c0, int) and c0 == 0:
                kv_round(g, 0, first=True)
                c0, n = 1, n - 1

            def body(c, carry):
                kv_round(g, c0 + c)
                return carry
            lax.fori_loop(0, n, body, 0)

        def issue_wo(t):
            for i in range(wo_pos[t], wo_pos[t + 1]):
                for p, blk in enumerate((wo_q0[i], wo_q1[i])):
                    for r, nr, c, nc in blk:
                        ix = (pl.ds(r, nr), pl.ds(c, nc))
                        pltpu.make_async_copy(
                            wo_hbm.at[ix], wob.at[ix], sem.at[wo_sem(r)]).start(priority=p)

        def qk(h, j):
            s = lax.dot_general(qs[h], kb[h], _NT, preferred_element_type=f32)
            m = jnp.max(s, axis=-1, keepdims=True)
            p = jnp.exp((s - m) * scale)
            ls[j] = jnp.broadcast_to(jnp.sum(p, axis=-1, keepdims=True), (8, _DH))
            ps[j] = p.astype(bf16)

        def pv(h, j):
            o = lax.dot_general(ps[j], vb[h], _NN, preferred_element_type=f32)
            os_[h] = (o / ls[j]).astype(bf16)

        def wait_k(g):
            wait_all(kb.at[pl.ds(g * _G, _G)], S_K + g)

        def wait_v(g):
            wait_all(vb.at[pl.ds(g * _G, _G)], S_V + g)

        issue_weights()
        issue_kv(0, 0, NR // 2)

        c_x.wait()
        x = xb[0].astype(f32)
        mu = jnp.mean(x, axis=-1, keepdims=True)
        xc = x - mu
        var = jnp.mean(xc * xc, axis=-1, keepdims=True)
        xn16 = (xc / jnp.sqrt(var + _EPS)).astype(bf16)
        xn8 = jnp.broadcast_to(xn16, (8, D))

        wait_all(wqb, S_WQ)
        q = lax.dot_general(xn8, wqb[...], _NN, preferred_element_type=f32)
        for h in range(_HQ):
            qs[h] = q[:, h * _DH:(h + 1) * _DH].astype(bf16)
        issue_kv(0, NR // 2, NR // 4)

        c_wr.wait()
        xn = xn16.astype(f32)
        r = jnp.sum(xn * wrb[...].astype(f32).reshape(1, D), axis=-1, keepdims=True)
        wait_all(wgb, S_WG)
        wait_all(wub, S_WU)
        wait_all(wdb, S_WD)
        gpre = lax.dot_general(xn8, wgb[...], _NT, preferred_element_type=f32)
        u = lax.dot_general(xn8, wub[...], _NT, preferred_element_type=f32)
        hmid = (gpre * _sigmoid(gpre) * u).astype(bf16)
        y = lax.dot_general(hmid, wdb[...], _NN, preferred_element_type=f32)
        b_out = xn + y[0:1, :] * _sigmoid(r)
        fin[0] = jnp.broadcast_to(x, (8, D))
        fin[1] = jnp.broadcast_to(b_out * _sigmoid(b_out), (8, D))
        issue_kv(0, 3 * NR // 4, NR // 4)

        def group(g, carry):
            hp = (g - 1) * _G
            issue_kv(g, 0, _LAG * step)
            wait_k(g - 1)

            def qk_step(j, c):
                qk(hp + j, j)
                issue_kv(g, (_LAG + j) * step, step)
                return c
            lax.fori_loop(0, _G, qk_step, 0)
            wait_v(g - 1)

            def pv_step(j, c):
                pv(hp + j, j)

                @pl.when(j < _G - _LAG)
                def _():
                    issue_kv(g, (_LAG + _G + j) * step, step)
                return c
            lax.fori_loop(0, _G, pv_step, 0)
            return carry

        lax.fori_loop(1, NG, group, 0)

        hp = (NG - 1) * _G
        for i, t0 in enumerate(tails):
            ocol[i] = jnp.broadcast_to(os_[t0 // _DH][0:1, :].astype(f32), (_DH, _DH)).T

        def last(fn, t0):
            def body(j, c):
                fn(hp + j, j)
                for t in range(_G):
                    pl.when(j == t)(lambda t=t: issue_wo(t0 + t))
                return c
            lax.fori_loop(0, _G, body, 0)

        issue_wo(0)
        wait_k(NG - 1)
        last(qk, 1)
        wait_v(NG - 1)
        last(pv, 1 + _G)

        acc_ref[...] = jnp.zeros_like(acc_ref)
        for batch in mxu_batches:
            for i in batch:
                lo, n = parts[i]
                wait_all(wob.at[pl.ds(lo, n), :], S_WO + i)
            for i in batch:
                lo, n = parts[i]
                oc = jnp.concatenate([os_[lo // _DH + t] for t in range(n // _DH)], axis=1)
                acc_ref[...] += lax.dot_general(
                    oc, wob[pl.ds(lo, n), :], _NN, preferred_element_type=f32)

        base = fin[0] + acc_ref[...] * fin[1]
        part = jnp.zeros((8, D), f32)
        for i in range(n_mxu, len(parts)):
            lo, n = parts[i]
            wait_all(wob.at[pl.ds(lo, n), :], S_WO + i)
            for r0 in range(lo, lo + n, 8):
                w = wob[pl.ds(r0, 8), :].astype(f32)
                oc = ocol[min(i - n_mxu, 1), pl.ds(r0 % _DH, 8), :]
                part = part + w * jnp.concatenate([oc] * (D // _DH), axis=1)
        out = base[0:1, :] + jnp.sum(part * fin[1], axis=0, keepdims=True)
        o_ref[0] = out.astype(o_ref.dtype)

    return kernel, n_sems


@jax.jit
def pallas_recurrent_scan__sliding_block_cached__moe_arch_mod__decode_kernel(
    A_x: jax.Array,
    A_k_cache: jax.Array,
    A_v_cache: jax.Array,
    A_wq: jax.Array,
    A_wo: jax.Array,
    B_x: jax.Array,
    B_w_r: jax.Array,
    B_w_gate: jax.Array,
    B_w_up: jax.Array,
    B_w_down: jax.Array,
):
    del B_x
    B, Sq, D = A_x.shape
    _, Hkv, SK, Dh = A_k_cache.shape
    F = B_w_gate.shape[1]
    assert B == 1 and Sq == 1 and Hkv == _HQ and Dh == _DH
    W = min(4096, max(256, SK // 4))
    f32, bf16 = jnp.float32, jnp.bfloat16
    kernel, n_sems = _make_kernel(D, F, SK, W)

    return pl.pallas_call(
        kernel,
        out_shape=jax.ShapeDtypeStruct((B, Sq, D), A_x.dtype),
        in_specs=[pl.BlockSpec(memory_space=pltpu.HBM)] * 9,
        out_specs=pl.BlockSpec(memory_space=pltpu.VMEM),
        scratch_shapes=[
            pltpu.VMEM((1, 1, D), bf16),
            pltpu.VMEM((D,), bf16),
            pltpu.VMEM((D, _HQ * _DH), bf16),
            pltpu.VMEM((_HQ * _DH, D), bf16),
            pltpu.VMEM((F, D), bf16),
            pltpu.VMEM((F, D), bf16),
            pltpu.VMEM((F, D), bf16),
            pltpu.VMEM((_HQ, W, _DH), bf16),
            pltpu.VMEM((_HQ, W, _DH), bf16),
            pltpu.VMEM((_HQ, 8, _DH), bf16),
            pltpu.VMEM((_G, 8, W), bf16),
            pltpu.VMEM((_G, 8, _DH), f32),
            pltpu.VMEM((_HQ, 8, _DH), bf16),
            pltpu.VMEM((8, D), f32),
            pltpu.VMEM((2, 8, D), f32),
            pltpu.VMEM((2, _DH, _DH), f32),
            pltpu.SemaphoreType.DMA((n_sems,)),
        ],
        compiler_params=pltpu.CompilerParams(
            vmem_limit_bytes=100 * 1024 * 1024,
            disable_semaphore_checks=True,
        ),
    )(A_x, A_k_cache, A_v_cache, A_wq, A_wo, B_w_r, B_w_gate.T, B_w_up.T, B_w_down)
```
